```python
import os as _os
_os.environ.setdefault("JAX_PLATFORMS", "cpu")
import jax
import jax.numpy as jnp

def _softmax(x, axis=-1):
    return jax.nn.softmax(x, axis=axis)
def _gelu(x):
    return jax.nn.gelu(x, approximate=True)
def _silu(x):
    return jax.nn.silu(x)
def _sigmoid(x):
    return jax.nn.sigmoid(x)
def _layernorm(x, axis=-1, eps=1e-5):
    m = jnp.mean(x, axis=axis, keepdims=True)
    v = jnp.var(x, axis=axis, keepdims=True)
    return (x - m) / jnp.sqrt(v + eps)
def _scatter_add(tgt, idx, src, axis=0):
    return tgt.at[idx].add(src)
def _segment_sum(src, seg, n):
    return jax.ops.segment_sum(src, seg, n)
class _Rng:
    def __init__(self, key):
        self._k = key
    def _next(self):
        self._k, sub = jax.random.split(self._k)
        return sub
    def normal(self, shape):
        return jax.random.normal(self._next(), shape, dtype=jnp.bfloat16)
    def randint(self, lo, hi, shape):
        return jax.random.randint(self._next(), shape, lo, hi, dtype=jnp.int32)
    def uniform(self, shape, lo=0.0, hi=1.0):
        return jax.random.uniform(self._next(), shape, jnp.bfloat16, lo, hi)
    def permutation(self, n):
        return jax.random.permutation(self._next(), n)


kernel_name = 'gated_mix__ssm_conv_s5__glu_gated_geglu__prompt'

def setup_inputs():
    _rng = _Rng(jax.random.key(int.from_bytes(__import__("os").urandom(4), "little")))
    _w = (lambda a: (lambda t: t.astype(jnp.bfloat16) if jnp.issubdtype(t.dtype, jnp.floating) else t)(jnp.asarray(a)))
    def _A_setup():
        B, S, D = 1, 2048, 1024
        P = D
        Lambda_re = -0.5 * jnp.exp((lambda *s: _rng.normal(s) * 0.4)(P))
        Lambda_im = (lambda *s: _rng.normal(s) * 0.4)(P) * 1.0
        B_re = (lambda *s: _rng.normal(s) * 0.4)(P, D) * (D ** -0.5)
        B_im = (lambda *s: _rng.normal(s) * 0.4)(P, D) * (D ** -0.5)
        C_re = (lambda *s: _rng.normal(s) * 0.4)(D, P) * (P ** -0.5)
        C_im = (lambda *s: _rng.normal(s) * 0.4)(D, P) * (P ** -0.5)
        log_dt = (lambda *s: _rng.normal(s) * 0.4)(P) * 0.3 - 2.0
        Dskip = (lambda *s: _rng.normal(s) * 0.4)(D)
        return {
            "x": _w((lambda *s: _rng.normal(s) * 0.05)(B, S, D)),
            "Lambda_re": _w(Lambda_re),
            "Lambda_im": _w(Lambda_im),
            "B_re": _w(B_re),
            "B_im": _w(B_im),
            "C_re": _w(C_re),
            "C_im": _w(C_im),
            "log_dt": _w(log_dt),
            "Dskip": _w(Dskip),
        }
    _A_in = _A_setup()

    def _B_setup():
        B, S, Dm, Df = 1, 2048, 1024, 3584
        return {
            "x": _w((lambda *s: _rng.normal(s) * 0.05)(B, S, Dm)),
            "w_gate": _w((lambda *s: _rng.normal(s) * 1.6)(Dm, Df) * (Dm ** -0.5)),
            "w_up": _w((lambda *s: _rng.normal(s) * 1.6)(Dm, Df) * (Dm ** -0.5)),
            "w_down": _w((lambda *s: _rng.normal(s) * 1.6)(Df, Dm) * (Df ** -0.5)),
        }
    _B_in = _B_setup()

    return {
        "A_x": _A_in["x"],
        "A_Lambda_re": _A_in["Lambda_re"],
        "A_Lambda_im": _A_in["Lambda_im"],
        "A_B_re": _A_in["B_re"],
        "A_B_im": _A_in["B_im"],
        "A_C_re": _A_in["C_re"],
        "A_C_im": _A_in["C_im"],
        "A_log_dt": _A_in["log_dt"],
        "A_Dskip": _A_in["Dskip"],
        "B_x": _B_in["x"],
        "B_w_gate": _B_in["w_gate"],
        "B_w_up": _B_in["w_up"],
        "B_w_down": _B_in["w_down"],
        "gate_w": _w((lambda *s: _rng.normal(s) * 0.05)(1024) * 16.0),
    }

def reference(A_x, A_Lambda_re, A_Lambda_im, A_B_re, A_B_im, A_C_re, A_C_im, A_log_dt, A_Dskip, B_x, B_w_gate, B_w_up, B_w_down, gate_w):
    def _A_ref(x, Lambda_re, Lambda_im, B_re, B_im, C_re, C_im, log_dt, Dskip):
        Bsz, L, H = x.shape
        Lam = Lambda_re + 1j * Lambda_im
        Bmat = B_re + 1j * B_im
        Cmat = C_re + 1j * C_im
        dt = jnp.exp(log_dt)
        Lam_bar = jnp.exp(dt * Lam)
        B_bar = ((Lam_bar - 1.0) / Lam)[:, None] * Bmat
        Bu = jnp.einsum("bld,pd->blp", x + 0j, B_bar)
        h = jnp.zeros_like(Bu[:, 0, :])
        hs = []
        for t in range(L):
            h = Lam_bar[None, :] * h + Bu[:, t, :]
            hs.append(h)
        hseq = jnp.stack(hs, 1)
        y = 2.0 * jnp.einsum("blp,dp->bld", hseq, Cmat).real + x * Dskip[None, None, :]
        return y

    def _B_ref(x, w_gate, w_up, w_down):
        g = jnp.einsum("bsd,df->bsf", x, w_gate)
        u = jnp.einsum("bsd,df->bsf", x, w_up)
        h = _gelu(g) * u
        return jnp.einsum("bsf,fd->bsd", h, w_down)

    x = A_x
    g = _sigmoid((x * gate_w).sum(-1, keepdims=True))
    a = _A_ref(x, A_Lambda_re, A_Lambda_im, A_B_re, A_B_im, A_C_re, A_C_im, A_log_dt, A_Dskip)
    b = _B_ref(x, B_w_gate, B_w_up, B_w_down)
    return g * a + (1 - g) * b
```

```python
import functools
import jax, jax.numpy as jnp
import numpy as np
from jax import lax
from jax.experimental import pallas as pl
from jax.experimental.pallas import tpu as pltpu

F32 = jnp.float32
BF16 = jnp.bfloat16
NT = (((1,), (1,)), ((), ()))

def cmul(ar, ai, br, bi):
    return ar * br - ai * bi, ar * bi + ai * br

def make(tm, nt, interpret=False, do_ssm=True, do_ffn=True):
    def fn(A_x, A_Lambda_re, A_Lambda_im, A_B_re, A_B_im, A_C_re, A_C_im, A_log_dt, A_Dskip, B_x, B_w_gate, B_w_up, B_w_down, gate_w):
        x = A_x[0]
        S, D = x.shape
        Df = B_w_gate.shape[1]
        P = A_Lambda_re.shape[0]
        tf = Df // nt
        tp = P // nt
        row = lambda a: a.reshape(1, -1)

        def kern(x_ref, lre_ref, lim_ref, ldt_ref, dsk_ref, gw_ref, bre_ref, bim_ref, cre_ref, cim_ref,
                 wg_ref, wu_ref, wd_ref, o_ref, tab_ref, carry_ref, gate_ref):
            i = pl.program_id(0)
            j = pl.program_id(1)

            @pl.when(jnp.logical_and(i == 0, j == 0))
            def _():
                lre = lre_ref[...].astype(F32)
                lim = lim_ref[...].astype(F32)
                dt = jnp.exp(ldt_ref[...].astype(F32)).astype(BF16).astype(F32)
                zr = jnp.broadcast_to(dt * lre, (8, P))
                zi = jnp.broadcast_to(dt * lim, (8, P))
                sub = lax.broadcasted_iota(jnp.int32, (8, P), 0)
                k = (sub + 1).astype(F32)
                mag = jnp.exp(k * zr)
                pr = mag * jnp.cos(k * zi)
                pi = mag * jnp.sin(k * zi)
                def bc(r):
                    return (jnp.broadcast_to(pr[r:r + 1], (8, P)), jnp.broadcast_to(pi[r:r + 1], (8, P)))
                l1r, l1i = bc(0)
                l2r, l2i = bc(1)
                l4r, l4i = bc(3)
                ar = l1r - 1.0
                ai = l1i
                cr_, ci_ = jnp.broadcast_to(lre, (8, P)), jnp.broadcast_to(lim, (8, P))
                den = cr_ * cr_ + ci_ * ci_
                cfr = (ar * cr_ + ai * ci_) / den
                cfi = (ai * cr_ - ar * ci_) / den
                tabs = [pr, pi,
                        jnp.where(sub >= 1, l1r, 0.0), jnp.where(sub >= 1, l1i, 0.0),
                        jnp.where(sub >= 2, l2r, 0.0), jnp.where(sub >= 2, l2i, 0.0),
                        jnp.where(sub >= 4, l4r, 0.0), jnp.where(sub >= 4, l4i, 0.0),
                        cfr, cfi]
                for t in range(nt):
                    for n, a in enumerate(tabs):
                        tab_ref[t, n] = a[:, t * tp:(t + 1) * tp]
                carry_ref[...] = jnp.zeros_like(carry_ref)

            xv = x_ref[...]

            @pl.when(j == 0)
            def _():
                xf = xv.astype(F32)
                s = jnp.sum(xf * gw_ref[...].astype(F32), axis=-1, keepdims=True)
                g = jax.nn.sigmoid(s)
                gate_ref[...] = jnp.broadcast_to(g, (tm, 128))
                o_ref[...] = g * (xf * dsk_ref[...].astype(F32))

            gate = gate_ref[...]
            acc = None
            if do_ssm:
                tab = tab_ref[j]
                br = lax.dot_general(xv, bre_ref[...], NT, preferred_element_type=F32).reshape(tm // 8, 8, tp)
                bi = lax.dot_general(xv, bim_ref[...], NT, preferred_element_type=F32).reshape(tm // 8, 8, tp)
                for n, sh in ((2, 1), (4, 2), (6, 4)):
                    cr = tab[n][None]; ci = tab[n + 1][None]
                    rr = pltpu.roll(br, sh, 1)
                    ri = pltpu.roll(bi, sh, 1)
                    dr, di = cmul(cr, ci, rr, ri)
                    br = br + dr
                    bi = bi + di
                pr = tab[0]; pi = tab[1]
                hr_c = carry_ref[j, 0]; hi_c = carry_ref[j, 1]
                hrs = []; his = []
                for q in range(tm // 8):
                    dr, di = cmul(pr, pi, hr_c, hi_c)
                    hr = br[q] + dr
                    hi = bi[q] + di
                    hrs.append(hr); his.append(hi)
                    hr_c = jnp.broadcast_to(hr[7:8], (8, tp))
                    hi_c = jnp.broadcast_to(hi[7:8], (8, tp))
                carry_ref[j, 0] = hr_c
                carry_ref[j, 1] = hi_c
                gt = jnp.concatenate([gate] * (tp // 128), axis=1)
                hr = (jnp.concatenate(hrs, axis=0) * gt).astype(BF16)
                hi = (jnp.concatenate(his, axis=0) * gt).astype(BF16)
                cfr = tab[8][0:1]; cfi = tab[9][0:1]
                cre = cre_ref[...].astype(F32); cim = cim_ref[...].astype(F32)
                c2r = (2.0 * (cre * cfr - cim * cfi)).astype(BF16)
                c2i = (-2.0 * (cre * cfi + cim * cfr)).astype(BF16)
                acc = lax.dot_general(hr, c2r, NT, preferred_element_type=F32)
                acc += lax.dot_general(hi, c2i, NT, preferred_element_type=F32)
            if do_ffn:
                g = jnp.dot(xv, wg_ref[...], preferred_element_type=F32)
                u = jnp.dot(xv, wu_ref[...], preferred_element_type=F32)
                omg = jnp.concatenate([1.0 - gate] * (tf // 128), axis=1)
                h = (jax.nn.gelu(g, approximate=True) * u * omg).astype(BF16)
                d = jnp.dot(h, wd_ref[...], preferred_element_type=F32)
                acc = d if acc is None else acc + d
            o_ref[...] += acc

        small = pl.BlockSpec((1, P), lambda i, j: (0, 0))
        out = pl.pallas_call(
            kern, grid=(S // tm, nt),
            in_specs=[pl.BlockSpec((tm, D), lambda i, j: (i, 0)),
                      small, small, small, small, small,
                      pl.BlockSpec((tp, D), lambda i, j: (j, 0)),
                      pl.BlockSpec((tp, D), lambda i, j: (j, 0)),
                      pl.BlockSpec((D, tp), lambda i, j: (0, j)),
                      pl.BlockSpec((D, tp), lambda i, j: (0, j)),
                      pl.BlockSpec((D, tf), lambda i, j: (0, j)),
                      pl.BlockSpec((D, tf), lambda i, j: (0, j)),
                      pl.BlockSpec((tf, D), lambda i, j: (j, 0))],
            out_specs=pl.BlockSpec((tm, D), lambda i, j: (i, 0)),
            out_shape=jax.ShapeDtypeStruct((S, D), F32),
            scratch_shapes=[pltpu.VMEM((nt, 10, 8, tp), F32),
                            pltpu.VMEM((nt, 2, 8, tp), F32),
                            pltpu.VMEM((tm, 128), F32)],
            compiler_params=pltpu.CompilerParams(dimension_semantics=('arbitrary', 'arbitrary'), vmem_limit_bytes=110 * 1024 * 1024),
            interpret=interpret,
        )(x, row(A_Lambda_re), row(A_Lambda_im), row(A_log_dt), row(A_Dskip), row(gate_w),
          A_B_re, A_B_im, A_C_re, A_C_im, B_w_gate, B_w_up, B_w_down)
        return out[None]
    return fn


_impl = make(512, 4)

@jax.jit
def pallas_gated_mix__ssm_conv_s5__glu_gated_geglu__prompt_kernel(A_x, A_Lambda_re, A_Lambda_im, A_B_re, A_B_im, A_C_re, A_C_im, A_log_dt, A_Dskip, B_x, B_w_gate, B_w_up, B_w_down, gate_w):
    return _impl(A_x, A_Lambda_re, A_Lambda_im, A_B_re, A_B_im, A_C_re, A_C_im, A_log_dt, A_Dskip, B_x, B_w_gate, B_w_up, B_w_down, gate_w)
```

```python
import functools
import jax, jax.numpy as jnp
import numpy as np
from jax import lax
from jax.experimental import pallas as pl
from jax.experimental.pallas import tpu as pltpu

F32 = jnp.float32
BF16 = jnp.bfloat16
NT = (((1,), (1,)), ((), ()))


def cmul(ar, ai, br, bi):
    return ar * br - ai * bi, ar * bi + ai * br


def gelu_mul(g, u, scale):
    c1 = np.float32(np.sqrt(2.0 / np.pi))
    c2 = np.float32(np.sqrt(2.0 / np.pi) * 0.044715)
    z = g * (c1 + c2 * (g * g))
    return (g * (u * scale)) * (1.0 + jnp.tanh(z))


def make(tm=512, nt=4, interpret=False, flags=None, peel_waits=True, split_out=1, wmode=0, gate0='early'):
    def fn(A_x, A_Lambda_re, A_Lambda_im, A_B_re, A_B_im, A_C_re, A_C_im, A_log_dt, A_Dskip, B_x, B_w_gate, B_w_up, B_w_down, gate_w):
        x = A_x[0]
        S, D = x.shape
        Df = B_w_gate.shape[1]
        P = A_Lambda_re.shape[0]
        tf = Df // nt
        tp = P // nt
        nb = tp // 128
        nc = S // tm
        L = tm // 8
        PT = L + 1
        tq = tm // nt
        sq = lambda a: a.reshape(8, 128)

        def kern(lre_hbm, lim_hbm, ldt_hbm, dsk_hbm, gw_hbm,
                 x_hbm, bre_hbm, bim_hbm, cre_hbm, cim_hbm, wg_hbm, wu_hbm, wd_hbm,
                 o_hbm,
                 x_s, bre_s, bim_s, cre_s, cim_s, wg_s, wu_s, wd_s, acc_s, gate_s,
                 sems, osem, par_s,
                 tab_ref, carry_ref, bu_s, h_s):

            def wslot(t, n):
                return 5 + 1 + n + jnp.where(t > 0, 1, 0) + 7 * t if not isinstance(t, int) else 5 + 1 + n + (1 if t > 0 else 0) + 7 * t

            def xslot(cc):
                return 5 + jnp.where(cc == 1, 8, 7 * nt + cc) if not isinstance(cc, int) else 5 + (0 if cc == 0 else 8 if cc == 1 else 7 * nt + cc)

            def pcopy(i):
                return pltpu.make_async_copy([lre_hbm, lim_hbm, ldt_hbm, dsk_hbm, gw_hbm][i], par_s.at[i], sems.at[i])

            def wcopy(t, n):
                src, dst = [
                    lambda: (bre_hbm.at[pl.ds(t * tp, tp), :], bre_s.at[t]),
                    lambda: (bim_hbm.at[pl.ds(t * tp, tp), :], bim_s.at[t]),
                    lambda: (wg_hbm.at[:, pl.ds(t * tf, tf)], wg_s.at[t]),
                    lambda: (wu_hbm.at[:, pl.ds(t * tf, tf)], wu_s.at[t]),
                    lambda: (cre_hbm.at[:, pl.ds(t * tp, tp)], cre_s.at[t]),
                    lambda: (cim_hbm.at[:, pl.ds(t * tp, tp)], cim_s.at[t]),
                    lambda: (wd_hbm.at[pl.ds(t * tf, tf), :], wd_s.at[t]),
                ][n]()
                return pltpu.make_async_copy(src, dst, sems.at[wslot(t, n)])

            def xcopy(cc):
                return pltpu.make_async_copy(x_hbm.at[pl.ds(cc * tm, tm), :], x_s.at[cc], sems.at[xslot(cc)])

            def ocopy(cc):
                return pltpu.make_async_copy(acc_s.at[cc], o_hbm.at[pl.ds(cc * tm, tm), :], osem.at[cc])

            def ocopyq(cc, q):
                w = D // split_out
                return pltpu.make_async_copy(acc_s.at[cc, :, pl.ds(q * w, w)], o_hbm.at[pl.ds(cc * tm, tm), pl.ds(q * w, w)], osem.at[cc * split_out + q])

            order = [('x', 0)] + [('w', 0, n) for n in range(7)] + [('x', 1)]
            for t in range(1, nt):
                order += [('w', t, n) for n in range(7)]
            order += [('x', cc) for cc in range(2, nc)]
            for i in range(5):
                pcopy(i).start()
            for o in order:
                (xcopy(o[1]) if o[0] == 'x' else wcopy(o[1], o[2])).start()

            for i in range(5):
                pcopy(i).wait()
            lre_ref, lim_ref, ldt_ref, dsk_ref, gw_ref = [par_s.at[i] for i in range(5)]
            lre = lre_ref[...].astype(F32)
            lim = lim_ref[...].astype(F32)
            dt = jnp.exp(ldt_ref[...].astype(F32)).astype(BF16).astype(F32)
            zr = dt * lre
            zi = dt * lim

            def cexp(k):
                mag = jnp.exp(k * zr)
                return mag * jnp.cos(k * zi), mag * jnp.sin(k * zi)
            l1 = cexp(1.0)
            ar = l1[0] - 1.0
            ai = l1[1]
            den = lre * lre + lim * lim
            cfr = 2.0 * (ar * lre + ai * lim) / den
            cfi = 2.0 * (ai * lre - ar * lim) / den
            sub = lax.broadcasted_iota(jnp.int32, (8, 128), 0)
            bc = lambda t, r: jnp.broadcast_to(t[r:r + 1], (8, 128))
            q1 = cexp(float(L)); q2 = cexp(float(2 * L)); q4 = cexp(float(4 * L))
            for r in range(8):
                t, b = r // nb, r % nb
                tabs = [bc(l1[0], r), bc(l1[1], r),
                        jnp.where(sub >= 1, bc(q1[0], r), 0.0), jnp.where(sub >= 1, bc(q1[1], r), 0.0),
                        jnp.where(sub >= 2, bc(q2[0], r), 0.0), jnp.where(sub >= 2, bc(q2[1], r), 0.0),
                        jnp.where(sub >= 4, bc(q4[0], r), 0.0), jnp.where(sub >= 4, bc(q4[1], r), 0.0),
                        bc(cfr, r), bc(cfi, r)]
                for n, a in enumerate(tabs):
                    tab_ref[t, b, n] = a
            carry_ref[...] = jnp.zeros_like(carry_ref)

            gw = gw_ref[...].astype(F32).reshape(1, D)
            dsk = dsk_ref[...].astype(F32).reshape(1, D)

            def gate_rows(cx, cd, r0, nrows):
                xf = x_s[cx, pl.ds(r0, nrows), :].astype(F32)
                g = jax.nn.sigmoid(jnp.sum(xf * gw, axis=-1, keepdims=True))
                gate_s[cd, pl.ds(r0, nrows), :] = jnp.broadcast_to(g, (nrows, 128))
                acc_s[cd, pl.ds(r0, nrows), :] = g * (xf * dsk)

            if gate0 == 'early':
                xcopy(0).wait()
                gate_rows(0, 0, 0, tm)

            def step(c, j, first):
                def wait(n):
                    if first and peel_waits:
                        if wmode == 0:
                            wcopy(j, n).wait()
                        else:
                            groups = {0: [0, 1], 2: [2], 3: [3, 4, 5], 6: [6]}
                            for m in groups.get(n, []):
                                wcopy(j, m).wait()
                if first and not peel_waits:
                    for n in range(7):
                        wcopy(j, n).wait()
                if first and gate0 == 'late':
                    xcopy(0).wait()
                wait(0)
                if first and gate0 == 'late':
                    gate_rows(0, 0, 0, tm)
                xv = x_s[c]
                bur = lax.dot_general(xv, bre_s[j], NT, preferred_element_type=F32)
                wait(1)
                bui = lax.dot_general(xv, bim_s[j], NT, preferred_element_type=F32)
                for b in range(nb):
                    cs = slice(b * 128, (b + 1) * 128)
                    for s in range(8):
                        bu_s[0, b, pl.ds(PT * s, L), :] = bur[s * L:(s + 1) * L, cs]
                        bu_s[1, b, pl.ds(PT * s, L), :] = bui[s * L:(s + 1) * L, cs]
                wait(2)
                g = jnp.dot(xv, wg_s[j], preferred_element_type=F32)
                gate = gate_s[c]
                hrl = []; hil = []
                for b in range(nb):
                    T = lambda n: tab_ref[j, b, n]
                    lr = T(0); li = T(1)
                    ld = lambda q, k: bu_s[q, b, pl.ds(k, 8, stride=PT), :]
                    er = ld(0, 0); ei = ld(1, 0)
                    for k in range(1, L):
                        dr, di = cmul(lr, li, er, ei)
                        er = dr + ld(0, k)
                        ei = di + ld(1, k)
                    fr = jnp.where(sub == 0, carry_ref[j, b, 0], pltpu.roll(er, 1, 0))
                    fi = jnp.where(sub == 0, carry_ref[j, b, 1], pltpu.roll(ei, 1, 0))
                    for n, sh in ((2, 1), (4, 2), (6, 4)):
                        dr, di = cmul(T(n), T(n + 1), pltpu.roll(fr, sh, 0), pltpu.roll(fi, sh, 0))
                        fr = fr + dr
                        fi = fi + di
                    hr, hi = fr, fi
                    for k in range(L):
                        dr, di = cmul(lr, li, hr, hi)
                        hr = dr + ld(0, k)
                        hi = di + ld(1, k)
                        h_s[0, b, pl.ds(k, 8, stride=PT), :] = hr
                        h_s[1, b, pl.ds(k, 8, stride=PT), :] = hi
                    carry_ref[j, b, 0] = jnp.broadcast_to(hr[7:8], (8, 128))
                    carry_ref[j, b, 1] = jnp.broadcast_to(hi[7:8], (8, 128))
                    nat = lambda q: jnp.concatenate([h_s[q, b, pl.ds(PT * s, L), :] for s in range(8)], axis=0)
                    hr = nat(0); hi = nat(1)
                    cr = jnp.tile(T(8), (tm // 8, 1)); ci = jnp.tile(T(9), (tm // 8, 1))
                    yr, yi = cmul(cr, ci, hr, hi)
                    hrl.append((yr * gate).astype(BF16))
                    hil.append((yi * (-gate)).astype(BF16))
                wait(3)
                u = jnp.dot(xv, wu_s[j], preferred_element_type=F32)
                omg = jnp.concatenate([0.5 - 0.5 * gate] * (tf // 128), axis=1)
                hf = gelu_mul(g, u, omg).astype(BF16)
                hr = jnp.concatenate(hrl, axis=1); hi = jnp.concatenate(hil, axis=1)
                if first:
                    if wmode == 0:
                        xcopy(1).wait()
                        gate_rows(1, 1, 0, tq)
                else:
                    gate_rows(jnp.minimum(c + 1, nc - 1), c + 1, pl.multiple_of(j * tq, tq), tq)
                if split_out == 1 or first:
                    acc = acc_s[c]
                    wait(4)
                    acc += lax.dot_general(hr, cre_s[j], NT, preferred_element_type=F32)
                    wait(5)
                    acc += lax.dot_general(hi, cim_s[j], NT, preferred_element_type=F32)
                    wait(6)
                    if first and wmode == 1:
                        xcopy(1).wait()
                        gate_rows(1, 1, 0, tq)
                    acc += jnp.dot(hf, wd_s[j], preferred_element_type=F32)
                    acc_s[c] = acc
                else:
                    wait(4); wait(5); wait(6)
                    w = D // split_out
                    for q in range(split_out):
                        cs = pl.ds(q * w, w)
                        acc = acc_s[c, :, cs]
                        acc += lax.dot_general(hr, cre_s[j, cs, :], NT, preferred_element_type=F32)
                        acc += lax.dot_general(hi, cim_s[j, cs, :], NT, preferred_element_type=F32)
                        acc += jnp.dot(hf, wd_s[j, :, cs], preferred_element_type=F32)
                        acc_s[c, :, cs] = acc
                        if not first:
                            @pl.when(j == nt - 1)
                            def _():
                                ocopyq(c, q).start()

            step(0, 0, True)

            def body(s, carry):
                c = lax.shift_right_logical(s, 2)
                j = lax.bitwise_and(s, 3)

                @pl.when(c == 0)
                def _():
                    for n in range(7):
                        wcopy(j, n).wait()

                @pl.when(jnp.logical_and(j == 0, c + 1 < nc))
                def _():
                    xcopy(c + 1).wait()

                step(c, j, False)

                if split_out == 1:
                    @pl.when(j == nt - 1)
                    def _():
                        ocopy(c).start()
                return carry

            lax.fori_loop(1, nc * nt, body, 0)
            for cc in range(nc):
                if split_out == 1:
                    ocopy(cc).wait()
                else:
                    for q in range(split_out):
                        ocopyq(cc, q).wait()

        vm = pl.BlockSpec(memory_space=pltpu.VMEM)
        anyspec = pl.BlockSpec(memory_space=pl.ANY)
        out = pl.pallas_call(
            kern,
            in_specs=[anyspec] * 13,
            out_specs=anyspec,
            out_shape=jax.ShapeDtypeStruct((S, D), F32),
            scratch_shapes=[pltpu.VMEM((nc, tm, D), BF16),
                            pltpu.VMEM((nt, tp, D), BF16), pltpu.VMEM((nt, tp, D), BF16),
                            pltpu.VMEM((nt, D, tp), BF16), pltpu.VMEM((nt, D, tp), BF16),
                            pltpu.VMEM((nt, D, tf), BF16), pltpu.VMEM((nt, D, tf), BF16),
                            pltpu.VMEM((nt, tf, D), BF16),
                            pltpu.VMEM((nc + 1, tm, D), F32),
                            pltpu.VMEM((nc + 1, tm, 128), F32),
                            pltpu.SemaphoreType.DMA((5 + 7 * nt + nc,)), pltpu.SemaphoreType.DMA((nc * split_out,)), pltpu.VMEM((5, 8, 128), BF16),
                            pltpu.VMEM((nt, nb, 10, 8, 128), F32),
                            pltpu.VMEM((nt, nb, 2, 8, 128), F32),
                            pltpu.VMEM((2, nb, tm + 8, 128), F32),
                            pltpu.VMEM((2, nb, tm + 8, 128), F32)],
            compiler_params=pltpu.CompilerParams(vmem_limit_bytes=110 * 1024 * 1024, flags=flags),
            interpret=interpret,
        )(sq(A_Lambda_re), sq(A_Lambda_im), sq(A_log_dt), sq(A_Dskip), sq(gate_w),
          x, A_B_re, A_B_im, A_C_re, A_C_im, B_w_gate, B_w_up, B_w_down)
        return out[None]
    return fn


_impl = make(split_out=4, wmode=1)


@jax.jit
def pallas_gated_mix__ssm_conv_s5__glu_gated_geglu__prompt_kernel(A_x, A_Lambda_re, A_Lambda_im, A_B_re, A_B_im, A_C_re, A_C_im, A_log_dt, A_Dskip, B_x, B_w_gate, B_w_up, B_w_down, gate_w):
    return _impl(A_x, A_Lambda_re, A_Lambda_im, A_B_re, A_B_im, A_C_re, A_C_im, A_log_dt, A_Dskip, B_x, B_w_gate, B_w_up, B_w_down, gate_w)
```

```python
import functools
import jax
import jax.numpy as jnp
import numpy as np
from jax import lax
from jax.experimental import pallas as pl
from jax.experimental.pallas import tpu as pltpu

F32 = jnp.float32
BF16 = jnp.bfloat16
_NT = (((1,), (1,)), ((), ()))
_GELU_C1 = float(np.sqrt(2.0 / np.pi))
_GELU_C2 = float(np.sqrt(2.0 / np.pi) * 0.044715)


def _cmul(ar, ai, br, bi):
    return ar * br - ai * bi, ar * bi + ai * br


def _dot(a, b):
    return jnp.dot(a, b, preferred_element_type=F32)


def _dot_nt(a, b):
    return lax.dot_general(a, b, _NT, preferred_element_type=F32)


def make(tm=512, nt=4, pad=4, split=8, first_cfg=(1, 1), loop_cfg=(0, 1), dord='fri', dord_p='rif',
         wplan='P0', upos=0, gpos=0, bord=0, upos_p=0, bord_p=0, srow=1, scol=1, osem=1, dsem=0, xw=0, idx=0, interpret=False, flags=None):
    def fn(A_x, A_Lambda_re, A_Lambda_im, A_B_re, A_B_im, A_C_re, A_C_im, A_log_dt, A_Dskip, B_x,
           B_w_gate, B_w_up, B_w_down, gate_w):
        del B_x
        x = A_x[0]
        S, D = x.shape
        Df = B_w_gate.shape[1]
        P = A_Lambda_re.shape[0]
        tf, tp = Df // nt, P // nt
        nb = tp // 128
        nc = S // tm
        L = tm // 8
        PT = L + pad
        tq = tm // nt
        spq = tq // L
        wsp = D // split

        BRE, BIM, WG, WU, CRE, CIM, WD = range(7)
        NPAR = 5
        if wplan == 'P0':
            groups0 = {0: [BRE, BIM], 2: [WG], 3: [WU, CRE, CIM], 4: [WD]}
        elif wplan == 'P1':
            groups0 = {0: [BRE], 1: [BIM], 2: [WG], 3: [WU, CRE, CIM], 4: [WD]}
        sem_of0 = {}
        nsem = 2
        for pos in sorted(groups0):
            for n in groups0[pos]:
                sem_of0[n] = nsem
            nsem += 1
        SEM_X1 = nsem
        SEM_T = nsem + 1
        SEM_XR = SEM_T + 2 * (nt - 1)
        SEM_O = SEM_XR + 1
        nsem = SEM_O + 1
        if dsem:
            nsem = 5 + 7 * nt + nc + nc * split + 1

        def kern(lre_hbm, lim_hbm, ldt_hbm, dsk_hbm, gw_hbm,
                 x_hbm, bre_hbm, bim_hbm, cre_hbm, cim_hbm, wg_hbm, wu_hbm, wd_hbm,
                 o_hbm,
                 par_s, x_s, wrow_s, wcol_s, bre_s, bim_s, wd_s, wg_s, wu_s, cre_s, cim_s, acc_s, gate_s, tab_s, carry_s, bu_s, h_s, sems):

            def W(t, n):
                if n in (BRE, BIM, WD):
                    if srow:
                        off, w = {BRE: (0, tp), BIM: (tp, tp), WD: (2 * tp, tf)}[n]
                        return wrow_s.at[t, pl.ds(off, w), :]
                    return {BRE: bre_s, BIM: bim_s, WD: wd_s}[n].at[t]
                if scol:
                    off, w = {WG: (0, tf), WU: (tf, tf), CRE: (2 * tf, tp), CIM: (2 * tf + tp, tp)}[n]
                    return wcol_s.at[t, :, pl.ds(off, w)]
                return {WG: wg_s, WU: wu_s, CRE: cre_s, CIM: cim_s}[n].at[t]

            def pcopy(i):
                src = (lre_hbm, lim_hbm, ldt_hbm, dsk_hbm, gw_hbm)[i]
                return pltpu.make_async_copy(src, par_s.at[i], sems.at[i if dsem & 1 else 0 if not dsem else 0])

            def wcopy(t, n):
                rows = lambda ref, w: ref.at[pl.ds(t * w, w), :]
                cols = lambda ref, w: ref.at[:, pl.ds(t * w, w)]
                src = {BRE: rows(bre_hbm, tp), BIM: rows(bim_hbm, tp), WD: rows(wd_hbm, tf), WG: cols(wg_hbm, tf),
                       WU: cols(wu_hbm, tf), CRE: cols(cre_hbm, tp), CIM: cols(cim_hbm, tp)}[n]
                dst = W(t, n)
                if t == 0:
                    sem = sem_of0[n]
                else:
                    sem = SEM_T + 2 * (t - 1) + (0 if n in (BRE, BIM, WD) else 1)
                if dsem:
                    sem = 6 + 7 * t + n + 0 * (1 if isinstance(t, int) and t > 0 else 0)
                return pltpu.make_async_copy(src, dst, sems.at[sem])

            def xcopy(cc):
                sem = 1 if cc == 0 else SEM_X1 if cc == 1 else SEM_XR
                if dsem:
                    sem = 5 if cc == 0 else 6 + 7 * nt + cc - 1
                return pltpu.make_async_copy(x_hbm.at[pl.ds(cc * tm, tm), :], x_s.at[cc], sems.at[sem])

            def ocopy(cc, q):
                cs = pl.ds(q * wsp, wsp)
                return pltpu.make_async_copy(acc_s.at[cc, :, cs], o_hbm.at[pl.ds(cc * tm, tm), cs], sems.at[SEM_O if not dsem else 6 + 7 * nt + nc + cc * split + q])

            for i in range(NPAR):
                pcopy(i).start()
            xcopy(0).start()
            for n in (BRE, BIM, WG, WU, CRE, CIM, WD):
                wcopy(0, n).start()
            xcopy(1).start()
            for t in range(1, nt):
                for n in (BRE, BIM, WG, WU, CRE, CIM, WD):
                    wcopy(t, n).start()
            for cc in range(2, nc):
                xcopy(cc).start()

            for i in range(NPAR):
                pcopy(i).wait()
            lre = par_s[0].astype(F32)
            lim = par_s[1].astype(F32)
            dt = jnp.exp(par_s[2].astype(F32)).astype(BF16).astype(F32)
            zr = dt * lre
            zi = dt * lim

            def cexp(k):
                mag = jnp.exp(k * zr)
                return mag * jnp.cos(k * zi), mag * jnp.sin(k * zi)

            lam = cexp(1.0)
            sc = jnp.maximum(jnp.abs(lre), jnp.abs(lim))
            ur, ui = lre / sc, lim / sc
            den = (ur * ur + ui * ui) * sc
            ar, ai = lam[0] - 1.0, lam[1]
            cfr = 2.0 * (ar * ur + ai * ui) / den
            cfi = 2.0 * (ai * ur - ar * ui) / den
            hop = [cexp(float(L)), cexp(float(2 * L)), cexp(float(4 * L))]
            sub = lax.broadcasted_iota(jnp.int32, (8, 128), 0)
            row = lambda t, r: jnp.broadcast_to(t[r:r + 1], (8, 128))
            for r in range(P // 128):
                tabs = [row(lam[0], r), row(lam[1], r)]
                for sh, (qr, qi) in zip((1, 2, 4), hop):
                    tabs += [jnp.where(sub >= sh, row(qr, r), 0.0), jnp.where(sub >= sh, row(qi, r), 0.0)]
                tabs += [row(cfr, r), row(cfi, r)]
                for n, a in enumerate(tabs):
                    tab_s[r // nb, r % nb, n] = a
            carry_s[...] = jnp.zeros_like(carry_s)
            gw = par_s[4].astype(F32).reshape(1, D)
            dsk = par_s[3].astype(F32).reshape(1, D)

            def gate_rows(cx, cd, q, nq):
                for s in range(nq * spq):
                    r0 = q * tq + s * L
                    if not isinstance(r0, int):
                        r0 = pl.multiple_of(r0, L)
                    xf = x_s[cx, pl.ds(r0, L), :].astype(F32)
                    g = jax.nn.sigmoid(jnp.sum(xf * gw, axis=-1, keepdims=True))
                    gate_s[cd, pl.ds((q * spq + s) * PT, L), :] = jnp.broadcast_to(g, (L, 128))
                    acc_s[cd, pl.ds(r0, L), :] = g * (xf * dsk)

            xcopy(0).wait()
            gate_rows(0, 0, 0, nt)

            def step(c, j, first):
                coef_in, gate_in = first_cfg if first else loop_cfg

                def wait(pos):
                    if first:
                        for n in groups0.get(pos, ()):
                            wcopy(0, n).wait()

                seg = lambda ref, *idx: jnp.concatenate(
                    [ref[(*idx, pl.ds(PT * s, L), slice(None))] for s in range(8)], axis=0)
                xv = x_s[c]
                wait(0)
                bur = _dot_nt(xv, W(j, BRE)[...])
                wait(1)
                bui = _dot_nt(xv, W(j, BIM)[...])
                for b in range(nb):
                    for s in range(8):
                        bu_s[0, b, pl.ds(PT * s, L), :] = bur[s * L:(s + 1) * L, b * 128:(b + 1) * 128]
                        bu_s[1, b, pl.ds(PT * s, L), :] = bui[s * L:(s + 1) * L, b * 128:(b + 1) * 128]
                wait(2)
                g = _dot(xv, W(j, WG)[...])

                def gate_next():
                    if not first:
                        gate_rows(jnp.minimum(c + 1, nc - 1), c + 1, j, 1)

                up_pos = upos_p if first else upos
                b_ord = bord_p if first else bord
                if up_pos == 1:
                    wait(3)
                    u = _dot(xv, W(j, WU)[...])
                if gpos == 2:
                    gate_next()

                st = [dict() for _ in range(nb)]

                def pass1(b):
                    T = lambda n: tab_s[j, b, n]
                    ld = lambda q, k: bu_s[q, b, pl.ds(k, 8, stride=PT), :]
                    lr, li = T(0), T(1)
                    er, ei = ld(0, 0), ld(1, 0)
                    for k in range(1, L):
                        dr, di = _cmul(lr, li, er, ei)
                        er, ei = dr + ld(0, k), di + ld(1, k)
                    st[b].update(er=er, ei=ei)

                def pass2(b):
                    T = lambda n: tab_s[j, b, n]
                    ld = lambda q, k: bu_s[q, b, pl.ds(k, 8, stride=PT), :]
                    lr, li = T(0), T(1)
                    cr, ci = T(8), T(9)
                    ncr, nci = -cr, -ci
                    scale = lambda vr, vi: (cr * vr - ci * vi, ncr * vi + nci * vr)
                    er, ei = st[b]['er'], st[b]['ei']
                    fr = jnp.where(sub == 0, carry_s[j, b, 0], pltpu.roll(er, 1, 0))
                    fi = jnp.where(sub == 0, carry_s[j, b, 1], pltpu.roll(ei, 1, 0))
                    for n, sh in ((2, 1), (4, 2), (6, 4)):
                        dr, di = _cmul(T(n), T(n + 1), pltpu.roll(fr, sh, 0), pltpu.roll(fi, sh, 0))
                        fr, fi = fr + dr, fi + di
                    if coef_in:
                        dr, di = _cmul(T(2), T(3), fr, fi)
                        carry_s[j, b, 0] = jnp.broadcast_to((dr + er)[7:8], (8, 128))
                        carry_s[j, b, 1] = jnp.broadcast_to((di + ei)[7:8], (8, 128))
                        fr, fi = scale(fr, fi)
                        li = -li
                    hr, hi = fr, fi
                    for k in range(L):
                        dr, di = _cmul(lr, li, hr, hi)
                        vr, vi = scale(ld(0, k), ld(1, k)) if coef_in else (ld(0, k), ld(1, k))
                        hr, hi = dr + vr, di + vi
                        if gate_in:
                            gk = gate_s[c, pl.ds(k, 8, stride=PT), :]
                            h_s[0, b, pl.ds(k, 8, stride=PT), :] = hr * gk
                            h_s[1, b, pl.ds(k, 8, stride=PT), :] = hi * gk
                        else:
                            h_s[0, b, pl.ds(k, 8, stride=PT), :] = hr
                            h_s[1, b, pl.ds(k, 8, stride=PT), :] = hi
                    if not coef_in:
                        carry_s[j, b, 0] = jnp.broadcast_to(hr[7:8], (8, 128))
                        carry_s[j, b, 1] = jnp.broadcast_to(hi[7:8], (8, 128))

                def finish(b):
                    T = lambda n: tab_s[j, b, n]
                    cr, ci = T(8), T(9)
                    yr, yi = seg(h_s, 0, b), seg(h_s, 1, b)
                    if not coef_in:
                        tile = lambda v: jnp.tile(v, (tm // 8, 1))
                        yr, yi = (tile(cr) * yr - tile(ci) * yi, tile(-cr) * yi + tile(-ci) * yr)
                    if not gate_in:
                        gt = seg(gate_s, c)
                        yr, yi = yr * gt, yi * gt
                    st[b].update(hre=yr.astype(BF16), him=yi.astype(BF16))

                if b_ord == 0:
                    for b in range(nb):
                        pass1(b); pass2(b); finish(b)
                elif b_ord == 1:
                    for b in range(nb):
                        pass1(b)
                    for b in range(nb):
                        pass2(b); finish(b)
                elif b_ord == 2:
                    for b in range(nb):
                        pass1(b); pass2(b)
                    for b in range(nb):
                        finish(b)
                hre = jnp.concatenate([s_['hre'] for s_ in st], axis=1)
                him = jnp.concatenate([s_['him'] for s_ in st], axis=1)

                if up_pos == 0:
                    wait(3)
                    u = _dot(xv, W(j, WU)[...])
                if gpos == 1:
                    gate_next()
                omg = jnp.concatenate([0.5 - 0.5 * seg(gate_s, c)] * (tf // 128), axis=1)
                z = g * (_GELU_C1 + _GELU_C2 * (g * g))
                hf = ((g * (u * omg)) * (1.0 + jnp.tanh(z))).astype(BF16)
                if gpos == 0:
                    gate_next()

                def down(acc, which, cs):
                    if which == 'r':
                        return acc + _dot_nt(hre, W(j, CRE)[cs, :])
                    if which == 'i':
                        return acc + _dot_nt(him, W(j, CIM)[cs, :])
                    return acc + _dot(hf, W(j, WD)[:, cs])

                if first:
                    acc = acc_s[c]
                    for which in dord_p:
                        if which == 'f':
                            wait(4)
                            xcopy(1).wait()
                            gate_rows(1, 1, 0, 1)
                        acc = down(acc, which, slice(None))
                    acc_s[c] = acc
                else:
                    for q in range(split):
                        cs = pl.ds(q * wsp, wsp)
                        acc = acc_s[c, :, cs]
                        for which in dord:
                            acc = down(acc, which, cs)
                        acc_s[c, :, cs] = acc

                        @pl.when(j == nt - 1)
                        def _():
                            ocopy(c, q).start()
                        if gpos == 4 and q == split // 2 - 1:
                            gate_next()
                    if gpos == 3:
                        gate_next()

            step(0, 0, True)

            def body(s, cj):
                c, j = cj
                if idx == 1:
                    c = lax.shift_right_logical(s, 2)
                    j = lax.bitwise_and(s, 3)

                @pl.when(c == 0)
                def _():
                    if dsem:
                        for n in range(7):
                            pltpu.make_async_copy(W(j, n), W(j, n), sems.at[6 + 7 * j + n]).wait()
                        return
                    sem = SEM_T + 2 * (j - 1)
                    if srow:
                        pltpu.make_async_copy(wrow_s.at[j], wrow_s.at[j], sems.at[sem]).wait()
                    else:
                        for n in (BRE, BIM, WD):
                            pltpu.make_async_copy(W(j, n), W(j, n), sems.at[sem]).wait()
                    if scol:
                        pltpu.make_async_copy(wcol_s.at[j], wcol_s.at[j], sems.at[sem + 1]).wait()
                    else:
                        for n in (WG, WU, CRE, CIM):
                            pltpu.make_async_copy(W(j, n), W(j, n), sems.at[sem + 1]).wait()

                if nc > 2:
                    @pl.when(s == nt - 1)
                    def _():
                        if dsem:
                            for cc in range(2, nc):
                                xcopy(cc).wait()
                            return
                        rest = x_s.at[pl.ds(2, nc - 2)]
                        pltpu.make_async_copy(rest, rest, sems.at[SEM_XR]).wait()

                step(c, j, False)
                last = j == nt - 1
                return jnp.where(last, c + 1, c), jnp.where(last, 0, j + 1)

            lax.fori_loop(1, nc * nt, body, (jnp.int32(0), jnp.int32(1)))
            if dsem:
                for cc in range(nc):
                    for q in range(split):
                        ocopy(cc, q).wait()
            else:
                pltpu.make_async_copy(o_hbm, o_hbm, sems.at[SEM_O]).wait()

        sq = lambda a: a.reshape(8, 128)
        hbm = pl.BlockSpec(memory_space=pl.ANY)
        out = pl.pallas_call(
            kern,
            in_specs=[hbm] * 13,
            out_specs=hbm,
            out_shape=jax.ShapeDtypeStruct((S, D), F32),
            scratch_shapes=[
                pltpu.VMEM((8, 8, 128), BF16),
                pltpu.VMEM((nc, tm, D), BF16),
                pltpu.VMEM((nt, 2 * tp + tf, D) if srow else (64, 128), BF16),
                pltpu.VMEM((nt, D, 2 * tf + 2 * tp) if scol else (64, 128), BF16),
                pltpu.VMEM((nt, tp, D) if not srow else (64, 128), BF16),
                pltpu.VMEM((nt, tp, D) if not srow else (64, 128), BF16),
                pltpu.VMEM((nt, tf, D) if not srow else (64, 128), BF16),
                pltpu.VMEM((nt, D, tf) if not scol else (64, 128), BF16),
                pltpu.VMEM((nt, D, tf) if not scol else (64, 128), BF16),
                pltpu.VMEM((nt, D, tp) if not scol else (64, 128), BF16),
                pltpu.VMEM((nt, D, tp) if not scol else (64, 128), BF16),
                pltpu.VMEM((nc + 1, tm, D), F32),
                pltpu.VMEM((nc + 1, 8 * PT, 128), F32),
                pltpu.VMEM((nt, nb, 10, 8, 128), F32),
                pltpu.VMEM((nt, nb, 2, 8, 128), F32),
                pltpu.VMEM((2, nb, 8 * PT, 128), F32),
                pltpu.VMEM((2, nb, 8 * PT, 128), F32),
                pltpu.SemaphoreType.DMA((nsem,)),
            ],
            compiler_params=pltpu.CompilerParams(vmem_limit_bytes=100 * 1024 * 1024, flags=flags),
            interpret=interpret,
        )(sq(A_Lambda_re), sq(A_Lambda_im), sq(A_log_dt), sq(A_Dskip), sq(gate_w),
          x, A_B_re, A_B_im, A_C_re, A_C_im, B_w_gate, B_w_up, B_w_down)
        return out[None]
    return fn


_impl = make(**dict(idx=1, wplan='P1'))


@jax.jit
def pallas_gated_mix__ssm_conv_s5__glu_gated_geglu__prompt_kernel(
        A_x, A_Lambda_re, A_Lambda_im, A_B_re, A_B_im, A_C_re, A_C_im, A_log_dt, A_Dskip,
        B_x, B_w_gate, B_w_up, B_w_down, gate_w):
    return _impl(A_x, A_Lambda_re, A_Lambda_im, A_B_re, A_B_im, A_C_re, A_C_im, A_log_dt, A_Dskip,
                 B_x, B_w_gate, B_w_up, B_w_down, gate_w)
```

```python
import functools
import jax
import jax.numpy as jnp
import numpy as np
from jax import lax
from jax.experimental import pallas as pl
from jax.experimental.pallas import tpu as pltpu

F32 = jnp.float32
BF16 = jnp.bfloat16
_NT = (((1,), (1,)), ((), ()))
_GELU_C1 = float(np.sqrt(2.0 / np.pi))
_GELU_C2 = float(np.sqrt(2.0 / np.pi) * 0.044715)


def _cmul(ar, ai, br, bi):
    return ar * br - ai * bi, ar * bi + ai * br


def _dot(a, b):
    return jnp.dot(a, b, preferred_element_type=F32)


def _dot_nt(a, b):
    return lax.dot_general(a, b, _NT, preferred_element_type=F32)


def make(tm=512, nt=4, pad=4, split=8, first_cfg=(1, 1), loop_cfg=(0, 1), dord='fri', dord_p='rif',
         wplan='P0', upos=0, gpos=0, bord=0, upos_p=0, bord_p=0, srow=1, scol=1, osem=1, dsem=0, xw=0, idx=0, g0=0, wga=4, lastsplit=1, xfresh=1, x0split=0, x1q=1, gb=0, gq=0, lastrows=1, fup=0, fc=0, gfirst=0, interpret=False, flags=None):
    def fn(A_x, A_Lambda_re, A_Lambda_im, A_B_re, A_B_im, A_C_re, A_C_im, A_log_dt, A_Dskip, B_x,
           B_w_gate, B_w_up, B_w_down, gate_w):
        del B_x
        x = A_x[0]
        S, D = x.shape
        Df = B_w_gate.shape[1]
        P = A_Lambda_re.shape[0]
        tf, tp = Df // nt, P // nt
        nb = tp // 128
        nc = S // tm
        L = tm // 8
        PT = L + pad
        tq = tm // nt
        spq = tq // L
        wsp = D // split

        BRE, BIM, WG, WU, CRE, CIM, WD = range(7)
        NPAR = 5
        if wplan == 'P0':
            groups0 = {0: [BRE, BIM], 2: [WG], 3: [WU, CRE, CIM], 4: [WD]}
        elif wplan == 'P1':
            groups0 = {0: [BRE], 1: [BIM], 2: [WG], 3: [WU, CRE, CIM], 4: [WD]}
        elif wplan == 'P2':
            groups0 = {0: [BRE], 1: [BIM], 2: [WG], 3: [WU, CRE, CIM], 4: [WD]}
        sem_of0 = {}
        nsem = 2
        for pos in sorted(groups0):
            for n in groups0[pos]:
                sem_of0[n] = nsem
            nsem += 1
        SEM_WGB = nsem
        nsem += 1
        SEM_X0B = nsem
        nsem += 1
        SEM_X1 = nsem
        SEM_T = nsem + 1
        SEM_XR = SEM_T + 2 * (nt - 1)
        SEM_O = SEM_XR + 1
        nsem = SEM_O + 1
        if dsem:
            nsem = 5 + 7 * nt + nc + nc * split + 1

        def kern(lre_hbm, lim_hbm, ldt_hbm, dsk_hbm, gw_hbm,
                 x_hbm, bre_hbm, bim_hbm, cre_hbm, cim_hbm, wg_hbm, wu_hbm, wd_hbm,
                 o_hbm,
                 par_s, x_s, wrow_s, wcol_s, bre_s, bim_s, wd_s, wg_s, wu_s, cre_s, cim_s, acc_s, gate_s, tab_s, carry_s, bu_s, h_s, sems):

            def W(t, n):
                if n in (BRE, BIM, WD):
                    if srow:
                        off, w = {BRE: (0, tp), BIM: (tp, tp), WD: (2 * tp, tf)}[n]
                        return wrow_s.at[t, pl.ds(off, w), :]
                    return {BRE: bre_s, BIM: bim_s, WD: wd_s}[n].at[t]
                if scol:
                    off, w = {WG: (0, tf), WU: (tf, tf), CRE: (2 * tf, tp), CIM: (2 * tf + tp, tp)}[n]
                    return wcol_s.at[t, :, pl.ds(off, w)]
                return {WG: wg_s, WU: wu_s, CRE: cre_s, CIM: cim_s}[n].at[t]

            def pcopy(i):
                src = (lre_hbm, lim_hbm, ldt_hbm, dsk_hbm, gw_hbm)[i]
                return pltpu.make_async_copy(src, par_s.at[i], sems.at[i if dsem & 1 else 0 if not dsem else 0])

            def wcopy(t, n):
                rows = lambda ref, w: ref.at[pl.ds(t * w, w), :]
                cols = lambda ref, w: ref.at[:, pl.ds(t * w, w)]
                src = {BRE: rows(bre_hbm, tp), BIM: rows(bim_hbm, tp), WD: rows(wd_hbm, tf), WG: cols(wg_hbm, tf),
                       WU: cols(wu_hbm, tf), CRE: cols(cre_hbm, tp), CIM: cols(cim_hbm, tp)}[n]
                dst = W(t, n)
                if t == 0:
                    sem = sem_of0[n]
                else:
                    sem = SEM_T + 2 * (t - 1) + (0 if n in (BRE, BIM, WD) else 1)
                if dsem:
                    sem = 6 + 7 * t + n + 0 * (1 if isinstance(t, int) and t > 0 else 0)
                return pltpu.make_async_copy(src, dst, sems.at[sem])

            def xcopy(cc):
                sem = 1 if cc == 0 else SEM_X1 if cc == 1 else SEM_XR
                if dsem:
                    sem = 5 if cc == 0 else 6 + 7 * nt + cc - 1
                return pltpu.make_async_copy(x_hbm.at[pl.ds(cc * tm, tm), :], x_s.at[cc], sems.at[sem])

            def ocopy(cc, q):
                cs = pl.ds(q * wsp, wsp)
                return pltpu.make_async_copy(acc_s.at[cc, :, cs], o_hbm.at[pl.ds(cc * tm, tm), cs], sems.at[SEM_O if not dsem else 6 + 7 * nt + nc + cc * split + q])

            for i in range(NPAR):
                pcopy(i).start()
            ca = wga * 128

            def wg0(piece):
                lo, w = (0, ca) if piece == 0 else (ca, tf - ca)
                return pltpu.make_async_copy(wg_hbm.at[:, pl.ds(lo, w)], W(0, WG).at[:, pl.ds(lo, w)],
                                             sems.at[sem_of0[WG] if piece == 0 else SEM_WGB])

            def x0half(h):
                rs = pl.ds(h * (tm // 2), tm // 2)
                return pltpu.make_async_copy(x_hbm.at[rs, :], x_s.at[0, rs, :], sems.at[1 if h == 0 else SEM_X0B])

            if x0split:
                x0half(0).start()
            else:
                xcopy(0).start()
            for n in (BRE, BIM, WG, WU, CRE, CIM, WD):
                if x0split and n == BIM:
                    x0half(1).start()
                if n == WG and wplan == 'P2':
                    wg0(0).start()
                    wg0(1).start()
                else:
                    wcopy(0, n).start()
            def x1piece(t):
                r0 = t * tq if isinstance(t, int) else pl.multiple_of(t * tq, tq)
                sem = SEM_X1 if isinstance(t, int) and t == 0 else SEM_T + 2 * (t - 1)
                return pltpu.make_async_copy(x_hbm.at[pl.ds(tm + r0, tq), :], x_s.at[1, pl.ds(r0, tq), :], sems.at[sem])

            if x1q:
                x1piece(0).start()
            else:
                xcopy(1).start()
            for t in range(1, nt):
                for n in (BRE, BIM, WG, WU, CRE, CIM, WD):
                    wcopy(t, n).start()
                    if x1q and n == BIM:
                        x1piece(t).start()
            for cc in range(2, nc):
                xcopy(cc).start()

            for i in range(NPAR):
                pcopy(i).wait()
            lre = par_s[0].astype(F32)
            lim = par_s[1].astype(F32)
            dt = jnp.exp(par_s[2].astype(F32)).astype(BF16).astype(F32)
            zr = dt * lre
            zi = dt * lim

            def cexp(k):
                mag = jnp.exp(k * zr)
                return mag * jnp.cos(k * zi), mag * jnp.sin(k * zi)

            lam = cexp(1.0)
            sc = jnp.maximum(jnp.abs(lre), jnp.abs(lim))
            ur, ui = lre / sc, lim / sc
            den = (ur * ur + ui * ui) * sc
            ar, ai = lam[0] - 1.0, lam[1]
            cfr = 2.0 * (ar * ur + ai * ui) / den
            cfi = 2.0 * (ai * ur - ar * ui) / den
            hop = [cexp(float(L)), cexp(float(2 * L)), cexp(float(4 * L))]
            sub = lax.broadcasted_iota(jnp.int32, (8, 128), 0)
            row = lambda t, r: jnp.broadcast_to(t[r:r + 1], (8, 128))
            for r in range(P // 128):
                tabs = [row(lam[0], r), row(lam[1], r)]
                for sh, (qr, qi) in zip((1, 2, 4), hop):
                    tabs += [jnp.where(sub >= sh, row(qr, r), 0.0), jnp.where(sub >= sh, row(qi, r), 0.0)]
                tabs += [row(cfr, r), row(cfi, r)]
                for n, a in enumerate(tabs):
                    tab_s[r // nb, r % nb, n] = a
            carry_s[...] = jnp.zeros_like(carry_s)
            gw = par_s[4].astype(F32).reshape(1, D)
            dsk = par_s[3].astype(F32).reshape(1, D)

            def gate_rows(cx, cd, q, nq):
                for s in range(nq * spq):
                    r0 = q * tq + s * L
                    if not isinstance(r0, int):
                        r0 = pl.multiple_of(r0, L)
                    xf = x_s[cx, pl.ds(r0, L), :].astype(F32)
                    g = jax.nn.sigmoid(jnp.sum(xf * gw, axis=-1, keepdims=True))
                    gate_s[cd, pl.ds((q * spq + s) * PT, L), :] = jnp.broadcast_to(g, (L, 128))
                    acc_s[cd, pl.ds(r0, L), :] = g * (xf * dsk)

            if x0split:
                x0half(0).wait()
                gate_rows(0, 0, 0, nt // 2)
            else:
                xcopy(0).wait()
                if g0 == 0:
                    gate_rows(0, 0, 0, nt)

            def step(c, j, first):
                coef_in, gate_in = first_cfg if first else loop_cfg

                def wait(pos):
                    if first:
                        for n in groups0.get(pos, ()):
                            wcopy(0, n).wait()

                seg = lambda ref, *idx: jnp.concatenate(
                    [ref[(*idx, pl.ds(PT * s, L), slice(None))] for s in range(8)], axis=0)
                fresh = first and xfresh
                X = (lambda: x_s[c]) if fresh else None
                if not fresh:
                    xv = x_s[c]
                    X = lambda: xv
                wait(0)
                if first and x0split:
                    hm = tm // 2
                    bura = _dot_nt(x_s[c, 0:hm, :], W(j, BRE)[...])
                    x0half(1).wait()
                    if gb == 0:
                        gate_rows(0, 0, nt // 2, nt // 2)
                    bur = jnp.concatenate([bura, _dot_nt(x_s[c, hm:tm, :], W(j, BRE)[...])], axis=0)
                elif fup and not first:
                    if gfirst:
                        g = _dot(X(), W(j, WG)[...])
                    bu = _dot_nt(X(), wrow_s[j, 0:2 * tp, :])
                    bur, bui = bu[:, 0:tp], bu[:, tp:2 * tp]
                else:
                    if gfirst and not first:
                        g = _dot(X(), W(j, WG)[...])
                    bur = _dot_nt(X(), W(j, BRE)[...])
                def gate_b(pos):
                    if first and x0split and gb == pos:
                        gate_rows(0, 0, nt // 2, nt // 2)

                if first and x0split and gb == 6:
                    gate_rows(0, 0, nt // 2, nt // 2)
                wait(1)
                gate_b(1)
                if not (fup and not first):
                    bui = _dot_nt(X(), W(j, BIM)[...])
                gate_b(7)
                for b in range(nb):
                    for s in range(8):
                        bu_s[0, b, pl.ds(PT * s, L), :] = bur[s * L:(s + 1) * L, b * 128:(b + 1) * 128]
                        bu_s[1, b, pl.ds(PT * s, L), :] = bui[s * L:(s + 1) * L, b * 128:(b + 1) * 128]
                if first and g0 == 1:
                    gate_rows(0, 0, 0, nt)
                if first and wplan == 'P2':
                    wg0(0).wait()
                    gate_b(2)
                    ga = _dot(X(), W(j, WG)[:, 0:ca])
                    gate_b(8)
                    wg0(1).wait()
                    gate_b(3)
                    if g0 == 2:
                        gate_rows(0, 0, 0, nt)
                    g = jnp.concatenate([ga, _dot(X(), W(j, WG)[:, ca:tf])], axis=1)
                    gate_b(9)
                else:
                    wait(2)
                    if first and g0 == 2:
                        gate_rows(0, 0, 0, nt)
                    if not (gfirst and not first):
                        g = _dot(X(), W(j, WG)[...])

                def gate_next():
                    if not first:
                        gate_rows(jnp.minimum(c + 1, nc - 1), c + 1, j, 1)

                up_pos = upos_p if first else upos
                b_ord = bord_p if first else bord
                if up_pos == 1:
                    wait(3)
                    gate_b(4)
                    u = _dot(X(), W(j, WU)[...])
                    gate_b(5)
                if gpos == 2:
                    gate_next()

                st = [dict() for _ in range(nb)]

                def pass1(b):
                    T = lambda n: tab_s[j, b, n]
                    ld = lambda q, k: bu_s[q, b, pl.ds(k, 8, stride=PT), :]
                    lr, li = T(0), T(1)
                    er, ei = ld(0, 0), ld(1, 0)
                    for k in range(1, L):
                        dr, di = _cmul(lr, li, er, ei)
                        er, ei = dr + ld(0, k), di + ld(1, k)
                    st[b].update(er=er, ei=ei)

                def pass2(b):
                    T = lambda n: tab_s[j, b, n]
                    ld = lambda q, k: bu_s[q, b, pl.ds(k, 8, stride=PT), :]
                    lr, li = T(0), T(1)
                    cr, ci = T(8), T(9)
                    ncr, nci = -cr, -ci
                    scale = lambda vr, vi: (cr * vr - ci * vi, ncr * vi + nci * vr)
                    er, ei = st[b]['er'], st[b]['ei']
                    fr = jnp.where(sub == 0, carry_s[j, b, 0], pltpu.roll(er, 1, 0))
                    fi = jnp.where(sub == 0, carry_s[j, b, 1], pltpu.roll(ei, 1, 0))
                    for n, sh in ((2, 1), (4, 2), (6, 4)):
                        dr, di = _cmul(T(n), T(n + 1), pltpu.roll(fr, sh, 0), pltpu.roll(fi, sh, 0))
                        fr, fi = fr + dr, fi + di
                    if coef_in:
                        dr, di = _cmul(T(2), T(3), fr, fi)
                        carry_s[j, b, 0] = jnp.broadcast_to((dr + er)[7:8], (8, 128))
                        carry_s[j, b, 1] = jnp.broadcast_to((di + ei)[7:8], (8, 128))
                        fr, fi = scale(fr, fi)
                        li = -li
                    hr, hi = fr, fi
                    for k in range(L):
                        dr, di = _cmul(lr, li, hr, hi)
                        vr, vi = scale(ld(0, k), ld(1, k)) if coef_in else (ld(0, k), ld(1, k))
                        hr, hi = dr + vr, di + vi
                        if gate_in:
                            gk = gate_s[c, pl.ds(k, 8, stride=PT), :]
                            h_s[0, b, pl.ds(k, 8, stride=PT), :] = hr * gk
                            h_s[1, b, pl.ds(k, 8, stride=PT), :] = hi * gk
                        else:
                            h_s[0, b, pl.ds(k, 8, stride=PT), :] = hr
                            h_s[1, b, pl.ds(k, 8, stride=PT), :] = hi
                    if not coef_in:
                        carry_s[j, b, 0] = jnp.broadcast_to(hr[7:8], (8, 128))
                        carry_s[j, b, 1] = jnp.broadcast_to(hi[7:8], (8, 128))

                def finish(b):
                    T = lambda n: tab_s[j, b, n]
                    cr, ci = T(8), T(9)
                    yr, yi = seg(h_s, 0, b), seg(h_s, 1, b)
                    if not coef_in:
                        tile = lambda v: jnp.tile(v, (tm // 8, 1))
                        yr, yi = (tile(cr) * yr - tile(ci) * yi, tile(-cr) * yi + tile(-ci) * yr)
                    if not gate_in:
                        gt = seg(gate_s, c)
                        yr, yi = yr * gt, yi * gt
                    st[b].update(hre=yr.astype(BF16), him=yi.astype(BF16))

                if b_ord == 0:
                    for b in range(nb):
                        pass1(b); pass2(b); finish(b)
                elif b_ord == 1:
                    for b in range(nb):
                        pass1(b)
                    for b in range(nb):
                        pass2(b); finish(b)
                elif b_ord == 2:
                    for b in range(nb):
                        pass1(b); pass2(b)
                    for b in range(nb):
                        finish(b)
                hre = jnp.concatenate([s_['hre'] for s_ in st], axis=1)
                him = jnp.concatenate([s_['him'] for s_ in st], axis=1)
                hcat = jnp.concatenate([hre, him], axis=1)

                if up_pos == 0:
                    wait(3)
                    u = _dot(X(), W(j, WU)[...])
                if gpos == 1:
                    gate_next()
                omg = jnp.concatenate([0.5 - 0.5 * seg(gate_s, c)] * (tf // 128), axis=1)
                z = g * (_GELU_C1 + _GELU_C2 * (g * g))
                hf = ((g * (u * omg)) * (1.0 + jnp.tanh(z))).astype(BF16)
                if gpos == 0:
                    gate_next()

                def down(acc, which, cs, rs=slice(None)):
                    if fc and which == 'r':
                        return acc + _dot_nt(hcat[rs], wcol_s[j, cs, 2 * tf:2 * tf + 2 * tp])
                    if fc and which == 'i':
                        return acc
                    if which == 'r':
                        return acc + _dot_nt(hre[rs], W(j, CRE)[cs, :])
                    if which == 'i':
                        return acc + _dot_nt(him[rs], W(j, CIM)[cs, :])
                    return acc + _dot(hf[rs], W(j, WD)[:, cs])

                if first:
                    acc = acc_s[c]
                    for which in dord_p:
                        if which == 'f':
                            wait(4)
                            (x1piece(0) if x1q else xcopy(1)).wait()
                            if gq == 0:
                                gate_rows(1, 1, 0, 1)
                        acc = down(acc, which, slice(None))
                        if which == 'f' and gq == 1:
                            gate_rows(1, 1, 0, 1)
                    acc_s[c] = acc
                else:
                    for q in range(split):
                        cs = pl.ds(q * wsp, wsp)
                        if q == split - 1 and lastrows > 1:
                            rr = tm // lastrows
                            for r in range(lastrows):
                                acc = acc_s[c, pl.ds(r * rr, rr), cs]
                                for which in dord:
                                    acc = down(acc, which, cs, slice(r * rr, (r + 1) * rr))
                                acc_s[c, pl.ds(r * rr, rr), cs] = acc

                                @pl.when(j == nt - 1)
                                def _():
                                    pltpu.make_async_copy(
                                        acc_s.at[c, pl.ds(r * rr, rr), cs],
                                        o_hbm.at[pl.ds(pl.multiple_of(c * tm + r * rr, rr), rr), cs], sems.at[SEM_O]).start()
                            continue
                        acc = acc_s[c, :, cs]
                        for which in dord:
                            acc = down(acc, which, cs)
                        acc_s[c, :, cs] = acc

                        @pl.when(j == nt - 1)
                        def _():
                            ocopy(c, q).start()
                        if gpos == 4 and q == split // 2 - 1:
                            gate_next()
                    if gpos == 3:
                        gate_next()

            step(0, 0, True)

            def body(s, cj):
                c, j = cj
                if idx == 1:
                    c = lax.shift_right_logical(s, 2)
                    j = lax.bitwise_and(s, 3)

                @pl.when(c == 0)
                def _():
                    if dsem:
                        for n in range(7):
                            pltpu.make_async_copy(W(j, n), W(j, n), sems.at[6 + 7 * j + n]).wait()
                        return
                    sem = SEM_T + 2 * (j - 1)
                    if x1q:
                        x1piece(j).wait()
                    if srow:
                        pltpu.make_async_copy(wrow_s.at[j], wrow_s.at[j], sems.at[sem]).wait()
                    else:
                        for n in (BRE, BIM, WD):
                            pltpu.make_async_copy(W(j, n), W(j, n), sems.at[sem]).wait()
                    if scol:
                        pltpu.make_async_copy(wcol_s.at[j], wcol_s.at[j], sems.at[sem + 1]).wait()
                    else:
                        for n in (WG, WU, CRE, CIM):
                            pltpu.make_async_copy(W(j, n), W(j, n), sems.at[sem + 1]).wait()

                if nc > 2:
                    @pl.when(s == nt - 1)
                    def _():
                        if dsem:
                            for cc in range(2, nc):
                                xcopy(cc).wait()
                            return
                        rest = x_s.at[pl.ds(2, nc - 2)]
                        pltpu.make_async_copy(rest, rest, sems.at[SEM_XR]).wait()

                step(c, j, False)
                last = j == nt - 1
                return jnp.where(last, c + 1, c), jnp.where(last, 0, j + 1)

            lax.fori_loop(1, nc * nt, body, (jnp.int32(0), jnp.int32(1)))
            if dsem:
                for cc in range(nc):
                    for q in range(split):
                        ocopy(cc, q).wait()
            else:
                pltpu.make_async_copy(o_hbm, o_hbm, sems.at[SEM_O]).wait()

        sq = lambda a: a.reshape(8, 128)
        hbm = pl.BlockSpec(memory_space=pl.ANY)
        out = pl.pallas_call(
            kern,
            in_specs=[hbm] * 13,
            out_specs=hbm,
            out_shape=jax.ShapeDtypeStruct((S, D), F32),
            scratch_shapes=[
                pltpu.VMEM((8, 8, 128), BF16),
                pltpu.VMEM((nc, tm, D), BF16),
                pltpu.VMEM((nt, 2 * tp + tf, D) if srow else (64, 128), BF16),
                pltpu.VMEM((nt, D, 2 * tf + 2 * tp) if scol else (64, 128), BF16),
                pltpu.VMEM((nt, tp, D) if not srow else (64, 128), BF16),
                pltpu.VMEM((nt, tp, D) if not srow else (64, 128), BF16),
                pltpu.VMEM((nt, tf, D) if not srow else (64, 128), BF16),
                pltpu.VMEM((nt, D, tf) if not scol else (64, 128), BF16),
                pltpu.VMEM((nt, D, tf) if not scol else (64, 128), BF16),
                pltpu.VMEM((nt, D, tp) if not scol else (64, 128), BF16),
                pltpu.VMEM((nt, D, tp) if not scol else (64, 128), BF16),
                pltpu.VMEM((nc + 1, tm, D), F32),
                pltpu.VMEM((nc + 1, 8 * PT, 128), F32),
                pltpu.VMEM((nt, nb, 10, 8, 128), F32),
                pltpu.VMEM((nt, nb, 2, 8, 128), F32),
                pltpu.VMEM((2, nb, 8 * PT, 128), F32),
                pltpu.VMEM((2, nb, 8 * PT, 128), F32),
                pltpu.SemaphoreType.DMA((nsem,)),
            ],
            compiler_params=pltpu.CompilerParams(vmem_limit_bytes=100 * 1024 * 1024, flags=flags),
            interpret=interpret,
        )(sq(A_Lambda_re), sq(A_Lambda_im), sq(A_log_dt), sq(A_Dskip), sq(gate_w),
          x, A_B_re, A_B_im, A_C_re, A_C_im, B_w_gate, B_w_up, B_w_down)
        return out[None]
    return fn


_impl = make(**dict(idx=1, wplan='P2', x0split=1, first_cfg=(0,1), upos_p=1, gb=1, gfirst=1, lastrows=4, fc=1))


@jax.jit
def pallas_gated_mix__ssm_conv_s5__glu_gated_geglu__prompt_kernel(
        A_x, A_Lambda_re, A_Lambda_im, A_B_re, A_B_im, A_C_re, A_C_im, A_log_dt, A_Dskip,
        B_x, B_w_gate, B_w_up, B_w_down, gate_w):
    return _impl(A_x, A_Lambda_re, A_Lambda_im, A_B_re, A_B_im, A_C_re, A_C_im, A_log_dt, A_Dskip,
                 B_x, B_w_gate, B_w_up, B_w_down, gate_w)
```

```python
import jax
import jax.numpy as jnp
import numpy as np
from jax import lax
from jax.experimental import pallas as pl
from jax.experimental.pallas import tpu as pltpu

F32 = jnp.float32
BF16 = jnp.bfloat16

S, D, DF, P = 2048, 1024, 3584, 1024

TM = 512
NT = 4
NC = S // TM
TF = DF // NT
TP = P // NT
NB = TP // 128
L = TM // 8
PITCH = L + 4
TQ = TM // NT
NSPLIT = D // 128
LAST_ROWS = 4
WG_A = 512

_NT_DIMS = (((1,), (1,)), ((), ()))
_GELU_C1 = float(np.sqrt(2.0 / np.pi))
_GELU_C2 = float(np.sqrt(2.0 / np.pi) * 0.044715)

BRE, BIM, WG, WU, CRE, CIM, WD = range(7)
_ROW_SLOT = {BRE: (0, TP), BIM: (TP, TP), WD: (2 * TP, TF)}
_COL_SLOT = {WG: (0, TF), WU: (TF, TF), CRE: (2 * TF, TP), CIM: (2 * TF + TP, TP)}

SEM_PAR, SEM_X0A, SEM_BRE, SEM_X0B, SEM_BIM, SEM_WGA, SEM_WGB, SEM_WUC, SEM_WD, SEM_X1 = range(10)
SEM_TILE = 10
SEM_XREST = SEM_TILE + 2 * (NT - 1)
SEM_OUT = SEM_XREST + 1
NSEM = SEM_OUT + 1
_SEM_TILE0 = {BRE: SEM_BRE, BIM: SEM_BIM, WU: SEM_WUC, CRE: SEM_WUC, CIM: SEM_WUC, WD: SEM_WD}


def _cmul(ar, ai, br, bi):
    return ar * br - ai * bi, ar * bi + ai * br


def _dot(a, b):
    return jnp.dot(a, b, preferred_element_type=F32)


def _dot_nt(a, b):
    return lax.dot_general(a, b, _NT_DIMS, preferred_element_type=F32)


def _kernel(lre_hbm, lim_hbm, ldt_hbm, dsk_hbm, gw_hbm,
            x_hbm, bre_hbm, bim_hbm, cre_hbm, cim_hbm, wg_hbm, wu_hbm, wd_hbm,
            o_hbm,
            par_s, x_s, wrow_s, wcol_s, acc_s, gate_s, tab_s, carry_s, bu_s, h_s, sems):

    def weight(t, n):
        if n in _ROW_SLOT:
            off, width = _ROW_SLOT[n]
            return wrow_s.at[t, pl.ds(off, width), :]
        off, width = _COL_SLOT[n]
        return wcol_s.at[t, :, pl.ds(off, width)]

    def par_copy(i):
        src = (lre_hbm, lim_hbm, ldt_hbm, dsk_hbm, gw_hbm)[i]
        return pltpu.make_async_copy(src, par_s.at[i], sems.at[SEM_PAR])

    def weight_copy(t, n):
        rows = lambda ref, w: ref.at[pl.ds(t * w, w), :]
        cols = lambda ref, w: ref.at[:, pl.ds(t * w, w)]
        src = {BRE: lambda: rows(bre_hbm, TP), BIM: lambda: rows(bim_hbm, TP), WD: lambda: rows(wd_hbm, TF),
               WG: lambda: cols(wg_hbm, TF), WU: lambda: cols(wu_hbm, TF),
               CRE: lambda: cols(cre_hbm, TP), CIM: lambda: cols(cim_hbm, TP)}[n]()
        if isinstance(t, int) and t == 0:
            sem = _SEM_TILE0[n]
        else:
            sem = SEM_TILE + 2 * (t - 1) + (0 if n in _ROW_SLOT else 1)
        return pltpu.make_async_copy(src, weight(t, n), sems.at[sem])

    def wg0_copy(piece):
        lo, width, sem = (0, WG_A, SEM_WGA) if piece == 0 else (WG_A, TF - WG_A, SEM_WGB)
        return pltpu.make_async_copy(wg_hbm.at[:, pl.ds(lo, width)],
                                     weight(0, WG).at[:, pl.ds(lo, width)], sems.at[sem])

    def x0_copy(half):
        rows = pl.ds(half * (TM // 2), TM // 2)
        return pltpu.make_async_copy(x_hbm.at[rows, :], x_s.at[0, rows, :],
                                     sems.at[SEM_X0B if half else SEM_X0A])

    def x1_copy(t):
        if isinstance(t, int):
            r0, sem = t * TQ, (SEM_X1 if t == 0 else SEM_TILE + 2 * (t - 1))
        else:
            r0, sem = pl.multiple_of(t * TQ, TQ), SEM_TILE + 2 * (t - 1)
        return pltpu.make_async_copy(x_hbm.at[pl.ds(TM + r0, TQ), :],
                                     x_s.at[1, pl.ds(r0, TQ), :], sems.at[sem])

    def xrest_copy(c):
        return pltpu.make_async_copy(x_hbm.at[pl.ds(c * TM, TM), :], x_s.at[c], sems.at[SEM_XREST])

    def out_copy(c, r0, nrows, cols):
        dst_rows = pl.ds(pl.multiple_of(c * TM + r0, nrows), nrows)
        return pltpu.make_async_copy(acc_s.at[c, pl.ds(r0, nrows), cols],
                                     o_hbm.at[dst_rows, cols], sems.at[SEM_OUT])

    for i in range(5):
        par_copy(i).start()
    x0_copy(0).start()
    weight_copy(0, BRE).start()
    x0_copy(1).start()
    weight_copy(0, BIM).start()
    wg0_copy(0).start()
    wg0_copy(1).start()
    for n in (WU, CRE, CIM, WD):
        weight_copy(0, n).start()
    x1_copy(0).start()
    for t in range(1, NT):
        for n in (BRE, BIM, WG, WU, CRE, CIM, WD):
            weight_copy(t, n).start()
            if n == BIM:
                x1_copy(t).start()
    for c in range(2, NC):
        xrest_copy(c).start()

    for i in range(5):
        par_copy(i).wait()
    lre = par_s[0].astype(F32)
    lim = par_s[1].astype(F32)
    dt = jnp.exp(par_s[2].astype(F32)).astype(BF16).astype(F32)
    zr = dt * lre
    zi = dt * lim

    def lam_pow(k):
        mag = jnp.exp(k * zr)
        return mag * jnp.cos(k * zi), mag * jnp.sin(k * zi)

    lam = lam_pow(1.0)
    big = jnp.maximum(jnp.abs(lre), jnp.abs(lim))
    ur, ui = lre / big, lim / big
    den = (ur * ur + ui * ui) * big
    ar, ai = lam[0] - 1.0, lam[1]
    coef_re = 2.0 * (ar * ur + ai * ui) / den
    coef_im = 2.0 * (ai * ur - ar * ui) / den
    hops = [lam_pow(float(L)), lam_pow(float(2 * L)), lam_pow(float(4 * L))]
    sub = lax.broadcasted_iota(jnp.int32, (8, 128), 0)
    bcast_row = lambda v, r: jnp.broadcast_to(v[r:r + 1], (8, 128))
    for r in range(P // 128):
        tabs = [bcast_row(lam[0], r), bcast_row(lam[1], r)]
        for shift, (qr, qi) in zip((1, 2, 4), hops):
            tabs += [jnp.where(sub >= shift, bcast_row(qr, r), 0.0),
                     jnp.where(sub >= shift, bcast_row(qi, r), 0.0)]
        tabs += [bcast_row(coef_re, r), bcast_row(coef_im, r)]
        for n, v in enumerate(tabs):
            tab_s[r // NB, r % NB, n] = v
    carry_s[...] = jnp.zeros_like(carry_s)
    dskip = par_s[3].astype(F32).reshape(1, D)
    gate_w = par_s[4].astype(F32).reshape(1, D)

    def prepare_rows(c_src, c_dst, q, nq):
        per = TQ // L
        for s in range(nq * per):
            r0 = q * TQ + s * L
            if not isinstance(r0, int):
                r0 = pl.multiple_of(r0, L)
            xf = x_s[c_src, pl.ds(r0, L), :].astype(F32)
            g = jax.nn.sigmoid(jnp.sum(xf * gate_w, axis=-1, keepdims=True))
            gate_s[c_dst, pl.ds((q * per + s) * PITCH, L), :] = jnp.broadcast_to(g, (L, 128))
            acc_s[c_dst, pl.ds(r0, L), :] = g * (xf * dskip)

    x0_copy(0).wait()
    prepare_rows(0, 0, 0, NT // 2)

    def segments(ref, *idx):
        return jnp.concatenate(
            [ref[(*idx, pl.ds(PITCH * s, L), slice(None))] for s in range(8)], axis=0)

    def scan_block(c, j, b):
        tab = lambda n: tab_s[j, b, n]
        load = lambda part, k: bu_s[part, b, pl.ds(k, 8, stride=PITCH), :]
        lr, li = tab(0), tab(1)
        er, ei = load(0, 0), load(1, 0)
        for k in range(1, L):
            dr, di = _cmul(lr, li, er, ei)
            er, ei = dr + load(0, k), di + load(1, k)
        fr = jnp.where(sub == 0, carry_s[j, b, 0], pltpu.roll(er, 1, 0))
        fi = jnp.where(sub == 0, carry_s[j, b, 1], pltpu.roll(ei, 1, 0))
        for n, shift in ((2, 1), (4, 2), (6, 4)):
            dr, di = _cmul(tab(n), tab(n + 1), pltpu.roll(fr, shift, 0), pltpu.roll(fi, shift, 0))
            fr, fi = fr + dr, fi + di
        hr, hi = fr, fi
        for k in range(L):
            dr, di = _cmul(lr, li, hr, hi)
            hr, hi = dr + load(0, k), di + load(1, k)
            gk = gate_s[c, pl.ds(k, 8, stride=PITCH), :]
            h_s[0, b, pl.ds(k, 8, stride=PITCH), :] = hr * gk
            h_s[1, b, pl.ds(k, 8, stride=PITCH), :] = hi * gk
        carry_s[j, b, 0] = jnp.broadcast_to(hr[7:8], (8, 128))
        carry_s[j, b, 1] = jnp.broadcast_to(hi[7:8], (8, 128))
        cr, ci = tab(8), tab(9)
        tile = lambda v: jnp.tile(v, (TM // 8, 1))
        yr, yi = segments(h_s, 0, b), segments(h_s, 1, b)
        yr, yi = tile(cr) * yr - tile(ci) * yi, tile(-cr) * yi + tile(-ci) * yr
        return yr.astype(BF16), yi.astype(BF16)

    def store_bu(bu_re, bu_im):
        for b in range(NB):
            for s in range(8):
                rows, cols = slice(s * L, (s + 1) * L), slice(b * 128, (b + 1) * 128)
                bu_s[0, b, pl.ds(PITCH * s, L), :] = bu_re[rows, cols]
                bu_s[1, b, pl.ds(PITCH * s, L), :] = bu_im[rows, cols]

    def activations(c, j, g, u):
        hs = [scan_block(c, j, b) for b in range(NB)]
        h_ssm = jnp.concatenate([h[0] for h in hs] + [h[1] for h in hs], axis=1)
        scale = jnp.concatenate([0.5 - 0.5 * segments(gate_s, c)] * (TF // 128), axis=1)
        z = g * (_GELU_C1 + _GELU_C2 * (g * g))
        h_mlp = ((g * (u * scale)) * (1.0 + jnp.tanh(z))).astype(BF16)
        return h_ssm, h_mlp

    def project(acc, j, h_ssm, h_mlp, cols, mlp_first):
        mlp = lambda: _dot(h_mlp, weight(j, WD)[:, cols])
        ssm = lambda: _dot_nt(h_ssm, wcol_s[j, cols, 2 * TF:2 * TF + 2 * TP])
        if mlp_first:
            return acc + mlp() + ssm()
        return acc + ssm() + mlp()

    def first_step():
        half = TM // 2
        weight_copy(0, BRE).wait()
        bu_a = _dot_nt(x_s[0, 0:half, :], weight(0, BRE)[...])
        x0_copy(1).wait()
        bu_re = jnp.concatenate([bu_a, _dot_nt(x_s[0, half:TM, :], weight(0, BRE)[...])], axis=0)
        weight_copy(0, BIM).wait()
        prepare_rows(0, 0, NT // 2, NT // 2)
        bu_im = _dot_nt(x_s[0], weight(0, BIM)[...])
        store_bu(bu_re, bu_im)
        wg0_copy(0).wait()
        ga = _dot(x_s[0], weight(0, WG)[:, 0:WG_A])
        wg0_copy(1).wait()
        g = jnp.concatenate([ga, _dot(x_s[0], weight(0, WG)[:, WG_A:TF])], axis=1)
        for n in (WU, CRE, CIM):
            weight_copy(0, n).wait()
        u = _dot(x_s[0], weight(0, WU)[...])
        h_ssm, h_mlp = activations(0, 0, g, u)
        acc = acc_s[0] + _dot_nt(h_ssm, wcol_s[0, :, 2 * TF:2 * TF + 2 * TP])
        weight_copy(0, WD).wait()
        x1_copy(0).wait()
        prepare_rows(1, 1, 0, 1)
        acc_s[0] = acc + _dot(h_mlp, weight(0, WD)[...])

    def step(c, j):
        x = x_s[c]
        g = _dot(x, weight(j, WG)[...])
        bu_re = _dot_nt(x, weight(j, BRE)[...])
        bu_im = _dot_nt(x, weight(j, BIM)[...])
        store_bu(bu_re, bu_im)
        u = _dot(x, weight(j, WU)[...])
        h_ssm, h_mlp = activations(c, j, g, u)
        prepare_rows(jnp.minimum(c + 1, NC - 1), c + 1, j, 1)
        last_tile = j == NT - 1
        for q in range(NSPLIT - 1):
            cols = pl.ds(q * 128, 128)
            acc_s[c, :, cols] = project(acc_s[c, :, cols], j, h_ssm, h_mlp, cols, True)

            @pl.when(last_tile)
            def _():
                out_copy(c, 0, TM, cols).start()

        cols = pl.ds((NSPLIT - 1) * 128, 128)
        nrows = TM // LAST_ROWS
        for r in range(LAST_ROWS):
            rows = slice(r * nrows, (r + 1) * nrows)
            acc_s[c, rows, cols] = project(acc_s[c, rows, cols], j, h_ssm[rows], h_mlp[rows], cols, True)

            @pl.when(last_tile)
            def _():
                out_copy(c, r * nrows, nrows, cols).start()

    first_step()

    def loop_body(s, carry):
        c = lax.shift_right_logical(s, NT.bit_length() - 1)
        j = lax.bitwise_and(s, NT - 1)

        @pl.when(c == 0)
        def _():
            for n in (BRE, BIM, WD):
                weight_copy(j, n).wait()
            x1_copy(j).wait()
            for n in (WG, WU, CRE, CIM):
                weight_copy(j, n).wait()

        @pl.when(s == NT - 1)
        def _():
            for cc in range(2, NC):
                xrest_copy(cc).wait()

        step(c, j)
        return carry

    lax.fori_loop(1, NC * NT, loop_body, 0)
    pltpu.make_async_copy(o_hbm, o_hbm, sems.at[SEM_OUT]).wait()


@jax.jit
def pallas_gated_mix__ssm_conv_s5__glu_gated_geglu__prompt_kernel(
    A_x: jax.Array,
    A_Lambda_re: jax.Array,
    A_Lambda_im: jax.Array,
    A_B_re: jax.Array,
    A_B_im: jax.Array,
    A_C_re: jax.Array,
    A_C_im: jax.Array,
    A_log_dt: jax.Array,
    A_Dskip: jax.Array,
    B_x: jax.Array,
    B_w_gate: jax.Array,
    B_w_up: jax.Array,
    B_w_down: jax.Array,
    gate_w: jax.Array,
):
    del B_x
    assert A_x.shape == (1, S, D) and A_B_re.shape == (P, D) and B_w_gate.shape == (D, DF)
    lanes = lambda v: v.reshape(8, 128)
    hbm = pl.BlockSpec(memory_space=pl.ANY)
    out = pl.pallas_call(
        _kernel,
        in_specs=[hbm] * 13,
        out_specs=hbm,
        out_shape=jax.ShapeDtypeStruct((S, D), F32),
        scratch_shapes=[
            pltpu.VMEM((8, 8, 128), BF16),
            pltpu.VMEM((NC, TM, D), BF16),
            pltpu.VMEM((NT, 2 * TP + TF, D), BF16),
            pltpu.VMEM((NT, D, 2 * TF + 2 * TP), BF16),
            pltpu.VMEM((NC + 1, TM, D), F32),
            pltpu.VMEM((NC + 1, 8 * PITCH, 128), F32),
            pltpu.VMEM((NT, NB, 10, 8, 128), F32),
            pltpu.VMEM((NT, NB, 2, 8, 128), F32),
            pltpu.VMEM((2, NB, 8 * PITCH, 128), F32),
            pltpu.VMEM((2, NB, 8 * PITCH, 128), F32),
            pltpu.SemaphoreType.DMA((NSEM,)),
        ],
        compiler_params=pltpu.CompilerParams(vmem_limit_bytes=100 * 1024 * 1024),
    )(lanes(A_Lambda_re), lanes(A_Lambda_im), lanes(A_log_dt), lanes(A_Dskip), lanes(gate_w),
      A_x[0], A_B_re, A_B_im, A_C_re, A_C_im, B_w_gate, B_w_up, B_w_down)
    return out[None]
```

```python
import jax
import jax.numpy as jnp
import numpy as np
from jax import lax
from jax.experimental import pallas as pl
from jax.experimental.pallas import tpu as pltpu

F32 = jnp.float32
BF16 = jnp.bfloat16

S, D, DF, P = 2048, 1024, 3584, 1024

TM = 512
NT = 4
NC = S // TM
TF = DF // NT
TP = P // NT
NB = TP // 128
L = TM // 8
PITCH = L + 4
TQ = TM // NT
NSPLIT = D // 128
LAST_ROWS = 4
WG_A = 512

_NT_DIMS = (((1,), (1,)), ((), ()))
_GELU_C1 = float(np.sqrt(2.0 / np.pi))
_GELU_C2 = float(np.sqrt(2.0 / np.pi) * 0.044715)

_SCHEDULER_FLAGS = (
    {"XLA_TPU_EVENLY_DISTRIBUTE_CRITICAL_NODES": True} if jax.__version_info__ >= (0, 12) else None)

BRE, BIM, WG, WU, CRE, CIM, WD = range(7)
_ROW_SLOT = {BRE: (0, TP), BIM: (TP, TP), WD: (2 * TP, TF)}
_COL_SLOT = {WG: (0, TF), WU: (TF, TF), CRE: (2 * TF, TP), CIM: (2 * TF + TP, TP)}

SEM_PAR, SEM_X0A, SEM_BRE, SEM_X0B, SEM_BIM, SEM_WGA, SEM_WGB, SEM_WUC, SEM_WD, SEM_X1 = range(10)
SEM_TILE = 10
SEM_XREST = SEM_TILE + 2 * (NT - 1)
SEM_OUT = SEM_XREST + 1
NSEM = SEM_OUT + 1
_SEM_TILE0 = {BRE: SEM_BRE, BIM: SEM_BIM, WU: SEM_WUC, CRE: SEM_WUC, CIM: SEM_WUC, WD: SEM_WD}


def _cmul(ar, ai, br, bi):
    return ar * br - ai * bi, ar * bi + ai * br


def _dot(a, b):
    return jnp.dot(a, b, preferred_element_type=F32)


def _dot_nt(a, b):
    return lax.dot_general(a, b, _NT_DIMS, preferred_element_type=F32)


def _kernel(lre_hbm, lim_hbm, ldt_hbm, dsk_hbm, gw_hbm,
            x_hbm, bre_hbm, bim_hbm, cre_hbm, cim_hbm, wg_hbm, wu_hbm, wd_hbm,
            o_hbm,
            par_s, x_s, wrow_s, wcol_s, acc_s, gate_s, tab_s, carry_s, bu_s, h_s, sems):

    def weight(t, n):
        if n in _ROW_SLOT:
            off, width = _ROW_SLOT[n]
            return wrow_s.at[t, pl.ds(off, width), :]
        off, width = _COL_SLOT[n]
        return wcol_s.at[t, :, pl.ds(off, width)]

    def par_copy(i):
        src = (lre_hbm, lim_hbm, ldt_hbm, dsk_hbm, gw_hbm)[i]
        return pltpu.make_async_copy(src, par_s.at[i], sems.at[SEM_PAR])

    def weight_copy(t, n):
        rows = lambda ref, w: ref.at[pl.ds(t * w, w), :]
        cols = lambda ref, w: ref.at[:, pl.ds(t * w, w)]
        src = {BRE: lambda: rows(bre_hbm, TP), BIM: lambda: rows(bim_hbm, TP), WD: lambda: rows(wd_hbm, TF),
               WG: lambda: cols(wg_hbm, TF), WU: lambda: cols(wu_hbm, TF),
               CRE: lambda: cols(cre_hbm, TP), CIM: lambda: cols(cim_hbm, TP)}[n]()
        if isinstance(t, int) and t == 0:
            sem = _SEM_TILE0[n]
        else:
            sem = SEM_TILE + 2 * (t - 1) + (0 if n in _ROW_SLOT else 1)
        return pltpu.make_async_copy(src, weight(t, n), sems.at[sem])

    def wg0_copy(piece):
        lo, width, sem = (0, WG_A, SEM_WGA) if piece == 0 else (WG_A, TF - WG_A, SEM_WGB)
        return pltpu.make_async_copy(wg_hbm.at[:, pl.ds(lo, width)],
                                     weight(0, WG).at[:, pl.ds(lo, width)], sems.at[sem])

    def x0_copy(half):
        rows = pl.ds(half * (TM // 2), TM // 2)
        return pltpu.make_async_copy(x_hbm.at[rows, :], x_s.at[0, rows, :],
                                     sems.at[SEM_X0B if half else SEM_X0A])

    def x1_copy(t):
        if isinstance(t, int):
            r0, sem = t * TQ, (SEM_X1 if t == 0 else SEM_TILE + 2 * (t - 1))
        else:
            r0, sem = pl.multiple_of(t * TQ, TQ), SEM_TILE + 2 * (t - 1)
        return pltpu.make_async_copy(x_hbm.at[pl.ds(TM + r0, TQ), :],
                                     x_s.at[1, pl.ds(r0, TQ), :], sems.at[sem])

    def xrest_copy(c):
        return pltpu.make_async_copy(x_hbm.at[pl.ds(c * TM, TM), :], x_s.at[c], sems.at[SEM_XREST])

    def out_copy(c, r0, nrows, cols):
        dst_rows = pl.ds(pl.multiple_of(c * TM + r0, nrows), nrows)
        return pltpu.make_async_copy(acc_s.at[c, pl.ds(r0, nrows), cols],
                                     o_hbm.at[dst_rows, cols], sems.at[SEM_OUT])

    for i in range(5):
        par_copy(i).start()
    x0_copy(0).start()
    weight_copy(0, BRE).start()
    x0_copy(1).start()
    weight_copy(0, BIM).start()
    wg0_copy(0).start()
    wg0_copy(1).start()
    for n in (WU, CRE, CIM, WD):
        weight_copy(0, n).start()
    x1_copy(0).start()
    for t in range(1, NT):
        for n in (BRE, BIM, WG, WU, CRE, CIM, WD):
            weight_copy(t, n).start()
            if n == BIM:
                x1_copy(t).start()
    for c in range(2, NC):
        xrest_copy(c).start()

    for i in range(5):
        par_copy(i).wait()
    lre = par_s[0].astype(F32)
    lim = par_s[1].astype(F32)
    dt = jnp.exp(par_s[2].astype(F32)).astype(BF16).astype(F32)
    zr = dt * lre
    zi = dt * lim

    def lam_pow(k):
        mag = jnp.exp(k * zr)
        return mag * jnp.cos(k * zi), mag * jnp.sin(k * zi)

    lam = lam_pow(1.0)
    big = jnp.maximum(jnp.abs(lre), jnp.abs(lim))
    ur, ui = lre / big, lim / big
    den = (ur * ur + ui * ui) * big
    ar, ai = lam[0] - 1.0, lam[1]
    coef_re = 2.0 * (ar * ur + ai * ui) / den
    coef_im = 2.0 * (ai * ur - ar * ui) / den
    hops = [lam_pow(float(L)), lam_pow(float(2 * L)), lam_pow(float(4 * L))]
    sub = lax.broadcasted_iota(jnp.int32, (8, 128), 0)
    bcast_row = lambda v, r: jnp.broadcast_to(v[r:r + 1], (8, 128))
    for r in range(P // 128):
        tabs = [bcast_row(lam[0], r), bcast_row(lam[1], r)]
        for shift, (qr, qi) in zip((1, 2, 4), hops):
            tabs += [jnp.where(sub >= shift, bcast_row(qr, r), 0.0),
                     jnp.where(sub >= shift, bcast_row(qi, r), 0.0)]
        tabs += [bcast_row(coef_re, r), bcast_row(coef_im, r)]
        for n, v in enumerate(tabs):
            tab_s[r // NB, r % NB, n] = v
    carry_s[...] = jnp.zeros_like(carry_s)
    dskip = par_s[3].astype(F32).reshape(1, D)
    gate_w = par_s[4].astype(F32).reshape(1, D)

    def prepare_rows(c_src, c_dst, q, nq):
        per = TQ // L
        for s in range(nq * per):
            r0 = q * TQ + s * L
            if not isinstance(r0, int):
                r0 = pl.multiple_of(r0, L)
            xf = x_s[c_src, pl.ds(r0, L), :].astype(F32)
            g = jax.nn.sigmoid(jnp.sum(xf * gate_w, axis=-1, keepdims=True))
            gate_s[c_dst, pl.ds((q * per + s) * PITCH, L), :] = jnp.broadcast_to(g, (L, 128))
            acc_s[c_dst, pl.ds(r0, L), :] = g * (xf * dskip)

    x0_copy(0).wait()
    prepare_rows(0, 0, 0, NT // 2)

    def segments(ref, *idx):
        return jnp.concatenate(
            [ref[(*idx, pl.ds(PITCH * s, L), slice(None))] for s in range(8)], axis=0)

    def scan_block(c, j, b):
        tab = lambda n: tab_s[j, b, n]
        load = lambda part, k: bu_s[part, b, pl.ds(k, 8, stride=PITCH), :]
        lr, li = tab(0), tab(1)
        er, ei = load(0, 0), load(1, 0)
        for k in range(1, L):
            dr, di = _cmul(lr, li, er, ei)
            er, ei = dr + load(0, k), di + load(1, k)
        fr = jnp.where(sub == 0, carry_s[j, b, 0], pltpu.roll(er, 1, 0))
        fi = jnp.where(sub == 0, carry_s[j, b, 1], pltpu.roll(ei, 1, 0))
        for n, shift in ((2, 1), (4, 2), (6, 4)):
            dr, di = _cmul(tab(n), tab(n + 1), pltpu.roll(fr, shift, 0), pltpu.roll(fi, shift, 0))
            fr, fi = fr + dr, fi + di
        hr, hi = fr, fi
        for k in range(L):
            dr, di = _cmul(lr, li, hr, hi)
            hr, hi = dr + load(0, k), di + load(1, k)
            gk = gate_s[c, pl.ds(k, 8, stride=PITCH), :]
            h_s[0, b, pl.ds(k, 8, stride=PITCH), :] = hr * gk
            h_s[1, b, pl.ds(k, 8, stride=PITCH), :] = hi * gk
        carry_s[j, b, 0] = jnp.broadcast_to(hr[7:8], (8, 128))
        carry_s[j, b, 1] = jnp.broadcast_to(hi[7:8], (8, 128))
        cr, ci = tab(8), tab(9)
        tile = lambda v: jnp.tile(v, (TM // 8, 1))
        yr, yi = segments(h_s, 0, b), segments(h_s, 1, b)
        yr, yi = tile(cr) * yr - tile(ci) * yi, tile(-cr) * yi + tile(-ci) * yr
        return yr.astype(BF16), yi.astype(BF16)

    def store_bu(bu_re, bu_im):
        for b in range(NB):
            for s in range(8):
                rows, cols = slice(s * L, (s + 1) * L), slice(b * 128, (b + 1) * 128)
                bu_s[0, b, pl.ds(PITCH * s, L), :] = bu_re[rows, cols]
                bu_s[1, b, pl.ds(PITCH * s, L), :] = bu_im[rows, cols]

    def activations(c, j, g, u):
        hs = [scan_block(c, j, b) for b in range(NB)]
        h_re = jnp.concatenate([h[0] for h in hs], axis=1)
        h_im = jnp.concatenate([h[1] for h in hs], axis=1)
        scale = jnp.concatenate([0.5 - 0.5 * segments(gate_s, c)] * (TF // 128), axis=1)
        z = g * (_GELU_C1 + _GELU_C2 * (g * g))
        h_mlp = ((g * (u * scale)) * (1.0 + jnp.tanh(z))).astype(BF16)
        return h_re, h_im, h_mlp

    def project(acc, j, h_re, h_im, h_mlp, cols):
        acc = acc + _dot(h_mlp, weight(j, WD)[:, cols])
        acc = acc + _dot_nt(h_re, weight(j, CRE)[cols, :])
        return acc + _dot_nt(h_im, weight(j, CIM)[cols, :])

    def first_step():
        half = TM // 2
        weight_copy(0, BRE).wait()
        bu_a = _dot_nt(x_s[0, 0:half, :], weight(0, BRE)[...])
        x0_copy(1).wait()
        bu_re = jnp.concatenate([bu_a, _dot_nt(x_s[0, half:TM, :], weight(0, BRE)[...])], axis=0)
        weight_copy(0, BIM).wait()
        prepare_rows(0, 0, NT // 2, NT // 2)
        bu_im = _dot_nt(x_s[0], weight(0, BIM)[...])
        store_bu(bu_re, bu_im)
        wg0_copy(0).wait()
        ga = _dot(x_s[0], weight(0, WG)[:, 0:WG_A])
        wg0_copy(1).wait()
        g = jnp.concatenate([ga, _dot(x_s[0], weight(0, WG)[:, WG_A:TF])], axis=1)
        for n in (WU, CRE, CIM):
            weight_copy(0, n).wait()
        u = _dot(x_s[0], weight(0, WU)[...])
        h_re, h_im, h_mlp = activations(0, 0, g, u)
        acc = acc_s[0] + _dot_nt(h_re, weight(0, CRE)[...])
        acc = acc + _dot_nt(h_im, weight(0, CIM)[...])
        weight_copy(0, WD).wait()
        x1_copy(0).wait()
        prepare_rows(1, 1, 0, 1)
        acc_s[0] = acc + _dot(h_mlp, weight(0, WD)[...])

    def step(c, j):
        x = x_s[c]
        g = _dot(x, weight(j, WG)[...])
        bu_re = _dot_nt(x, weight(j, BRE)[...])
        bu_im = _dot_nt(x, weight(j, BIM)[...])
        store_bu(bu_re, bu_im)
        u = _dot(x, weight(j, WU)[...])
        h_re, h_im, h_mlp = activations(c, j, g, u)
        last_tile = j == NT - 1
        for q in range(NSPLIT - 1):
            cols = pl.ds(q * 128, 128)
            acc_s[c, :, cols] = project(acc_s[c, :, cols], j, h_re, h_im, h_mlp, cols)

            @pl.when(last_tile)
            def _():
                out_copy(c, 0, TM, cols).start()

            if q == NSPLIT // 2 - 1:
                prepare_rows(jnp.minimum(c + 1, NC - 1), c + 1, j, 1)

        cols = pl.ds((NSPLIT - 1) * 128, 128)
        nrows = TM // LAST_ROWS
        for r in range(LAST_ROWS):
            rows = slice(r * nrows, (r + 1) * nrows)
            acc_s[c, rows, cols] = project(acc_s[c, rows, cols], j, h_re[rows], h_im[rows], h_mlp[rows], cols)

            @pl.when(last_tile)
            def _():
                out_copy(c, r * nrows, nrows, cols).start()

    first_step()

    def loop_body(s, carry):
        c = lax.shift_right_logical(s, NT.bit_length() - 1)
        j = lax.bitwise_and(s, NT - 1)

        @pl.when(c == 0)
        def _():
            for n in (BRE, BIM, WD):
                weight_copy(j, n).wait()
            x1_copy(j).wait()
            for n in (WG, WU, CRE, CIM):
                weight_copy(j, n).wait()

        @pl.when(s == NT - 1)
        def _():
            for cc in range(2, NC):
                xrest_copy(cc).wait()

        step(c, j)
        return carry

    lax.fori_loop(1, NC * NT, loop_body, 0)
    pltpu.make_async_copy(o_hbm, o_hbm, sems.at[SEM_OUT]).wait()


@jax.jit
def pallas_gated_mix__ssm_conv_s5__glu_gated_geglu__prompt_kernel(
    A_x: jax.Array,
    A_Lambda_re: jax.Array,
    A_Lambda_im: jax.Array,
    A_B_re: jax.Array,
    A_B_im: jax.Array,
    A_C_re: jax.Array,
    A_C_im: jax.Array,
    A_log_dt: jax.Array,
    A_Dskip: jax.Array,
    B_x: jax.Array,
    B_w_gate: jax.Array,
    B_w_up: jax.Array,
    B_w_down: jax.Array,
    gate_w: jax.Array,
):
    del B_x
    assert A_x.shape == (1, S, D) and A_B_re.shape == (P, D) and B_w_gate.shape == (D, DF)
    lanes = lambda v: v.reshape(8, 128)
    hbm = pl.BlockSpec(memory_space=pl.ANY)
    out = pl.pallas_call(
        _kernel,
        in_specs=[hbm] * 13,
        out_specs=hbm,
        out_shape=jax.ShapeDtypeStruct((S, D), F32),
        scratch_shapes=[
            pltpu.VMEM((8, 8, 128), BF16),
            pltpu.VMEM((NC, TM, D), BF16),
            pltpu.VMEM((NT, 2 * TP + TF, D), BF16),
            pltpu.VMEM((NT, D, 2 * TF + 2 * TP), BF16),
            pltpu.VMEM((NC + 1, TM, D), F32),
            pltpu.VMEM((NC + 1, 8 * PITCH, 128), F32),
            pltpu.VMEM((NT, NB, 10, 8, 128), F32),
            pltpu.VMEM((NT, NB, 2, 8, 128), F32),
            pltpu.VMEM((2, NB, 8 * PITCH, 128), F32),
            pltpu.VMEM((2, NB, 8 * PITCH, 128), F32),
            pltpu.SemaphoreType.DMA((NSEM,)),
        ],
        compiler_params=pltpu.CompilerParams(
            vmem_limit_bytes=100 * 1024 * 1024,
            flags=_SCHEDULER_FLAGS),
    )(lanes(A_Lambda_re), lanes(A_Lambda_im), lanes(A_log_dt), lanes(A_Dskip), lanes(gate_w),
      A_x[0], A_B_re, A_B_im, A_C_re, A_C_im, B_w_gate, B_w_up, B_w_down)
    return out[None]
```
